```python
import jax
import jax.numpy as jnp

def _softmax(x, axis=-1):
    return jax.nn.softmax(x, axis=axis)
def _gelu(x):
    return jax.nn.gelu(x, approximate=True)
def _silu(x):
    return jax.nn.silu(x)
def _sigmoid(x):
    return jax.nn.sigmoid(x)
def _layernorm(x, axis=-1, eps=1e-5):
    m = jnp.mean(x, axis=axis, keepdims=True)
    v = jnp.var(x, axis=axis, keepdims=True)
    return (x - m) / jnp.sqrt(v + eps)
def _scatter_add(tgt, idx, src, axis=0):
    return tgt.at[idx].add(src)
def _segment_sum(src, seg, n):
    return jax.ops.segment_sum(src, seg, n)
class _Rng:
    def __init__(self, key):
        self._k = key
    def _next(self):
        self._k, sub = jax.random.split(self._k)
        return sub
    def normal(self, shape):
        return jax.random.normal(self._next(), shape, dtype=jnp.bfloat16)
    def randint(self, lo, hi, shape):
        return jax.random.randint(self._next(), shape, lo, hi, dtype=jnp.int32)
    def uniform(self, shape, lo=0.0, hi=1.0):
        return jax.random.uniform(self._next(), shape, jnp.bfloat16, lo, hi)
    def permutation(self, n):
        return jax.random.permutation(self._next(), n)


kernel_name = 'parallel_sum__linear_kernel_hedgehog__glu_gated_geglu__prompt'

def _fwd_setup_inputs():
    _rng = _Rng(jax.random.key(int.from_bytes(__import__("os").urandom(4), "little")))
    _w = (lambda a: (lambda t: t.astype(jnp.bfloat16) if jnp.issubdtype(t.dtype, jnp.floating) else t)(jnp.asarray(a)))
    def _A_setup():
        B, S, D, H = 1, 2048, 448, 16
        Dh = D // H
        return {
            "x": _w((lambda *s: _rng.normal(s) * 0.05)(B, S, D)),
            "wqkv": _w((lambda *s: _rng.normal(s) * 0.05)(D, 3 * D)),
            "w_phi": _w((lambda *s: _rng.normal(s) * 0.05)(H, Dh, Dh) * (Dh ** -0.5)),
            "wo": _w((lambda *s: _rng.normal(s) * 0.05)(D, D)),
        }
    _A_in = _A_setup()

    def _B_setup():
        B, S, Dm, Df = 1, 2048, 448, 1792
        return {
            "x": _w((lambda *s: _rng.normal(s) * 0.05)(B, S, Dm)),
            "w_gate": _w((lambda *s: _rng.normal(s) * 0.05)(Dm, Df) * (Dm ** -0.5)),
            "w_up": _w((lambda *s: _rng.normal(s) * 0.05)(Dm, Df) * (Dm ** -0.5)),
            "w_down": _w((lambda *s: _rng.normal(s) * 0.05)(Df, Dm) * (Df ** -0.5)),
        }
    _B_in = _B_setup()

    return {
        "A_x": _A_in["x"],
        "A_wqkv": _A_in["wqkv"],
        "A_w_phi": _A_in["w_phi"],
        "A_wo": _A_in["wo"],
        "B_x": _B_in["x"],
        "B_w_gate": _B_in["w_gate"],
        "B_w_up": _B_in["w_up"],
        "B_w_down": _B_in["w_down"],
    }

def _fwd_reference(A_x, A_wqkv, A_w_phi, A_wo, B_x, B_w_gate, B_w_up, B_w_down):
    def _A_ref(x, wqkv, w_phi, wo):
        B, S, D = x.shape
        H = 16; Dh = D // H
        qkv = (lambda x, *d: x.transpose(*d))((x @ wqkv).reshape(B, S, 3, H, Dh), 2, 0, 3, 1, 4)
        q, k, v = qkv[0], qkv[1], qkv[2]
        pq = jnp.einsum("bhsd,hdf->bhsf", q, w_phi)
        pk = jnp.einsum("bhsd,hdf->bhsf", k, w_phi)
        phi_q = jnp.concatenate([_softmax(pq, axis=-1), _softmax(-pq, axis=-1)], axis=-1)
        phi_k = jnp.concatenate([_softmax(pk, axis=-1), _softmax(-pk, axis=-1)], axis=-1)
        kv = jnp.einsum("bhsf,bhsd->bhfd", phi_k, v)
        z  = jnp.einsum("bhsf->bhf", phi_k)
        num = jnp.einsum("bhqf,bhfd->bhqd", phi_q, kv)
        den = jnp.einsum("bhqf,bhf->bhq", phi_q, z)[..., None] + 1e-6
        o = num / den
        return (lambda x, *d: x.transpose(*d))(o, 0, 2, 1, 3).reshape(B, S, D) @ wo

    def _B_ref(x, w_gate, w_up, w_down):
        g = jnp.einsum("bsd,df->bsf", x, w_gate)
        u = jnp.einsum("bsd,df->bsf", x, w_up)
        h = _gelu(g) * u
        return jnp.einsum("bsf,fd->bsd", h, w_down)

    x = A_x
    xn = _layernorm(x, axis=-1)
    return x + _A_ref(xn, A_wqkv, A_w_phi, A_wo) + _B_ref(xn, B_w_gate, B_w_up, B_w_down)


def setup_inputs():
    _inp = _fwd_setup_inputs()
    _gk = jax.random.fold_in(jax.random.key(int.from_bytes(__import__("os").urandom(4), "little")), 2**31 - 1)
    _shapes = [[1, 2048, 448]]
    _dtypes = ['bfloat16']
    _gks = jax.random.split(_gk, len(_shapes))
    _gs = [jax.random.normal(k, s, dtype=jnp.dtype(d)) * 0.05 for k, s, d in zip(_gks, _shapes, _dtypes)]
    _inp["grad_out"] = _gs[0]
    return _inp

def reference(A_x, A_wqkv, A_w_phi, A_wo, B_w_gate, B_w_up, B_w_down, B_x, grad_out):
    _const = dict(B_x=B_x)
    def _f(*_d):
        return _fwd_reference(**{'A_x': _d[0], 'A_wqkv': _d[1], 'A_w_phi': _d[2], 'A_wo': _d[3], 'B_w_gate': _d[4], 'B_w_up': _d[5], 'B_w_down': _d[6], **_const})
    _out, _vjp = jax.vjp(_f, A_x, A_wqkv, A_w_phi, A_wo, B_w_gate, B_w_up, B_w_down)
    _grads = _vjp(grad_out)
    _out0 = jnp.asarray(_out)
    return (_out0, *[jnp.asarray(_g) for _g in _grads])
```

```python
import jax
import jax.numpy as jnp
import jax.experimental.pallas as pl
import jax.experimental.pallas.tpu as pltpu
from jax import lax

S = 2048
D = 448
F = 1792
H = 16
DH = 28
NG = 4
GR = 112
T = 512
NT = S // T
TS = 256
FC = 256
NC = F // FC
RS = 16
DD = D // 2
BF = jnp.bfloat16
F32 = jnp.float32
LN_EPS = 1e-5
DEN_EPS = 1e-6
GELU_C0 = 0.7978845608028654
GELU_C1 = 0.044715


def _nn(a, b):
    return lax.dot_general(a, b, (((1,), (0,)), ((), ())), preferred_element_type=F32)


def _nt(a, b):
    return lax.dot_general(a, b, (((1,), (1,)), ((), ())), preferred_element_type=F32)


def _iota(shape, dim):
    return lax.broadcasted_iota(jnp.int32, shape, dim)


def _div28(r):
    return (r * 9363) >> 18


def _fold(x, op):
    r = op(x, axis=0)
    rr = pltpu.roll(r, 4, 0)
    if op is jnp.max:
        return jnp.maximum(r, rr)
    if op is jnp.min:
        return jnp.minimum(r, rr)
    return r + rr


def _softmax_pm(p):
    n = p.shape[-1]
    p3 = p.reshape(14, 8, n)
    mx = _fold(p3, jnp.max)
    mn = _fold(p3, jnp.min)
    ep = jnp.exp(p3 - mx[None])
    em = jnp.exp(mn[None] - p3)
    rp = 1.0 / _fold(ep, jnp.sum)
    rm = 1.0 / _fold(em, jnp.sum)
    return ep, em, rp, rm


def _b_sums(x):
    b11, b12, b21, b22 = x[:DD, :TS], x[:DD, TS:], x[DD:, :TS], x[DD:, TS:]
    return [b11 + b22, b12 - b22, b21 - b11, b11 + b12, b21 + b22]


def _b_get(bs, full, t, r):
    if r == 1:
        return full[t, :DD, :TS]
    if r == 4:
        return full[t, DD:, TS:]
    return bs[t, {0: 0, 2: 1, 3: 2, 5: 3, 6: 4}[r]]


def _a_list(w):
    w11, w12, w21, w22 = w[:DD, :128], w[:DD, 128:], w[DD:, :128], w[DD:, 128:]
    f = lambda z: z.astype(F32)
    return [(f(w11) + f(w22)).astype(BF), (f(w12) + f(w22)).astype(BF), w11, w22,
            (f(w11) + f(w21)).astype(BF), (f(w12) - f(w11)).astype(BF), (f(w21) - f(w22)).astype(BF)]


def _c_list(c11, c12, c21, c22):
    return [z.astype(BF) for z in (c11 + c22, c21 - c22, c12 + c22, c11 + c21, c12 - c11, c22, c11)]


def _p_combine(p, t):
    top = jnp.concatenate([p[t, 0] + p[t, 1] - p[t, 3] + p[t, 5], p[t, 2] + p[t, 5]], axis=1)
    bot = jnp.concatenate([p[t, 3] + p[t, 6], p[t, 0] - p[t, 2] + p[t, 4] + p[t, 6]], axis=1)
    return jnp.concatenate([top, bot], axis=0)


def _q_combine(q):
    top = jnp.concatenate([q[0] + q[2] + q[4] - q[5], q[1] + q[5]], axis=1)
    bot = jnp.concatenate([q[4] + q[6], q[0] + q[1] + q[3] - q[6]], axis=1)
    return jnp.concatenate([top, bot], axis=0)


def _kt_rows(w):
    w1, w2 = w[:, :128], w[:, 128:]
    dz = (w1[256:384].astype(F32) - w2[256:384].astype(F32))
    a = jnp.concatenate([w1[:256], dz[64:].astype(BF), w1[384:]], axis=0)
    b = jnp.concatenate([w2[:256], (-dz[:64]).astype(BF), w2[384:]], axis=0)
    y = jnp.concatenate([w1[256:320], w2[320:384]], axis=0)
    return a.T, b.T, y.T


def _kt_dot(a, b, y, x):
    yy = _nn(y, x[256:384])
    o1 = _nn(a, jnp.concatenate([x[:256], x[320:]], axis=0)) + yy
    o2 = _nn(b, jnp.concatenate([x[:320], x[384:]], axis=0)) + yy
    return o1, o2


def _kernel(xT_h, wqkv_h, wphi_h, wo_h, wg_h, wu_h, wdT_h, dyT_h,
            out_h, dx_h, dwqkv_h, dwphi_h, dwo_h, dwg_h, dwu_h, dwdT_h,
            xT, dyT, wqkv, wphi, wo, wgu, wdT,
            xnT, rstd, dxT, doT, phik, vaug,
            wT, woT, wa, wpqT, wpq, wc, bd,
            kv, kvb, kvT, zb, dkv, dkvb, dkvT, gqT, gvk, dwo_acc,
            bx, bdy, pout, pdx, la, lb, ly, ch, cgu,
            out_o, dx_o, dwqkv_o, dwphi_o, dwo_o, dwgu_o, dwd_o, dwqkT,
            s_x, s_dy, s_w, s_g, s_u, s_d, so_out, so_dx, so_w, so_g, so_u, so_d):
    cp = pltpu.make_async_copy

    def tok(t):
        return pl.ds(pl.multiple_of(t * T, T), T)

    def fch(c):
        return pl.ds(pl.multiple_of(c * FC, FC), FC)

    def cx(t):
        return cp(xT_h.at[:, tok(t)], xT.at[t], s_x.at[t])

    def cdy(t):
        return cp(dyT_h.at[:, tok(t)], dyT.at[t], s_dy.at[t])

    def cg(c):
        return cp(wg_h.at[:, fch(c)], wgu.at[c, :, pl.ds(0, FC)], s_g.at[c])

    def cu(c):
        return cp(wu_h.at[:, fch(c)], wgu.at[c, :, pl.ds(FC, FC)], s_u.at[c])

    def cd(c):
        return cp(wdT_h.at[:, fch(c)], wdT.at[c], s_d.at[c])

    c_wo = cp(wo_h, wo, s_w.at[0])
    c_wphi = cp(wphi_h, wphi, s_w.at[1])
    c_wqkv = cp(wqkv_h, wqkv, s_w.at[2])

    def o_out(t):
        return cp(out_o.at[t], out_h.at[:, tok(t)], so_out.at[t])

    def o_dx(t):
        return cp(dx_o.at[t], dx_h.at[:, tok(t)], so_dx.at[t])

    def o_g(c):
        return cp(dwgu_o.at[c, :, pl.ds(0, FC)], dwg_h.at[:, fch(c)], so_g.at[c])

    def o_u(c):
        return cp(dwgu_o.at[c, :, pl.ds(FC, FC)], dwu_h.at[:, fch(c)], so_u.at[c])

    def o_d(c):
        return cp(dwd_o.at[c], dwdT_h.at[:, fch(c)], so_d.at[c])

    o_wqkv = cp(dwqkv_o, dwqkv_h, so_w.at[0])
    o_wphi = cp(dwphi_o, dwphi_h, so_w.at[1])
    o_wo = cp(dwo_o, dwo_h, so_w.at[2])

    c_wphi.start()
    c_wqkv.start()
    cx(0).start()
    c_wo.start()
    cdy(0).start()
    for t in range(1, NT):
        cx(t).start()
        cdy(t).start()
    for c in range(NC):
        cg(c).start(priority=1)
        cu(c).start(priority=1)
        cd(c).start(priority=1)

    with jax.named_scope("prep"):
        c_wphi.wait()
        pw = wphi[...].reshape(DH * H, DH)
        e_m = (_iota((DH, GR), 0) == (_iota((DH, GR), 1) >> 2)).astype(F32).astype(BF)
        q_m = _nn(pw, e_m)
        keep = (_iota((D, GR), 0) & 3) == (_iota((D, GR), 1) & 3)
        q_m = jnp.where(keep, q_m, 0.0).astype(BF)
        r_i = _iota((D, D), 0)
        r_h = _div28(r_i)
        perm = (_iota((D, D), 1) == (r_i - r_h * DH) * H + r_h).astype(F32).astype(BF)
        bd_all = _nn(perm, q_m)
        bd[...] = bd_all.astype(BF)
        c_wqkv.wait()
        wT[...] = wqkv[...].T
        for g in range(NG):
            bdt = bd_all[g * GR:(g + 1) * GR, :].T.astype(BF)
            wa[g * GR:(g + 1) * GR, :] = _nn(bdt, wT[D + g * GR:D + (g + 1) * GR, :]).astype(BF)
            wpqT[g * GR:(g + 1) * GR, :] = _nn(bdt, wT[g * GR:(g + 1) * GR, :]).astype(BF)
        wa[D:, :] = wT[2 * D:, :]
        wpq[...] = wpqT[...].T
        wc[...] = jnp.concatenate([wa[D:, :], wa[:D, :]], axis=0).T
        c_wo.wait()
        woT[...] = wo[...].T
        kv[...] = jnp.zeros_like(kv)
        dkv[...] = jnp.zeros_like(dkv)
        gqT[...] = jnp.zeros_like(gqT)
        gvk[...] = jnp.zeros_like(gvk)
        dwo_acc[...] = jnp.zeros_like(dwo_acc)

    def phase_a(t, carry):
        cx(t).wait()
        cdy(t).wait()
        subs = [slice(s * TS, (s + 1) * TS) for s in range(T // TS)]
        xns = []
        xfs = []
        for sl in subs:
            x = xT[t, :, sl].astype(F32)
            mu = jnp.sum(x, axis=0, keepdims=True) * (1.0 / D)
            xc = x - mu
            var = jnp.sum(xc * xc, axis=0, keepdims=True) * (1.0 / D)
            rs = lax.rsqrt(var + LN_EPS)
            xf = xc * rs
            xn = xf.astype(BF)
            xnT[t, :, sl] = xn
            rstd[t, :, sl] = jnp.broadcast_to(rs, (8, TS))
            xns.append(xn)
            xfs.append(xf)
        for i, z in enumerate(_b_sums(jnp.concatenate(xfs, axis=1))):
            bx[t, i] = z.astype(BF)
        for i, z in enumerate(_b_sums(dyT[t].astype(F32))):
            bdy[t, i] = z.astype(BF)
        pout[t] = jnp.zeros((7, DD, TS), F32)
        pdx[t] = jnp.zeros((7, DD, TS), F32)
        doT[t] = _nn(wo[...], dyT[t]).astype(BF)
        ones = jnp.ones((16, TS), BF)
        for sl, xn in zip(subs, xns):
            pv = _nn(wa[...], xn)
            for g in range(NG):
                ep, em, rp, rm = _softmax_pm(pv[g * GR:(g + 1) * GR])
                phik[t, g * 2 * GR:g * 2 * GR + GR, sl] = (ep * rp[None]).reshape(GR, TS).astype(BF)
                phik[t, g * 2 * GR + GR:(g + 1) * 2 * GR, sl] = (em * rm[None]).reshape(GR, TS).astype(BF)
                vaug[t, g * 128:g * 128 + GR, sl] = pv[D + g * GR:D + (g + 1) * GR].astype(BF)
                vaug[t, g * 128 + GR:(g + 1) * 128, sl] = ones
        for g in range(NG):
            kv[g] += _nt(phik[t, g * 2 * GR:(g + 1) * 2 * GR, :], vaug[t, g * 128:(g + 1) * 128, :])
        return carry

    with jax.named_scope("phaseA"):
        lax.fori_loop(0, NT, phase_a, 0)

    def prep_l(c):
        for i, w in enumerate((wgu[c, :, :FC], wgu[c, :, FC:], wdT[c])):
            a, b, y = _kt_rows(w)
            la[i * 128:(i + 1) * 128, :] = a
            lb[i * 128:(i + 1) * 128, :] = b
            ly[i * 128:(i + 1) * 128, :] = y

    row_j = _iota((2 * GR, 128), 0) & 3
    col = _iota((2 * GR, 128), 1)
    same_head = (row_j == _div28(col)) & (col < GR)

    with jax.named_scope("midA"):
        for g in range(NG):
            a = kv[g]
            am = jnp.where(same_head, a, 0.0)
            kvb[g] = am[:, :GR].astype(BF)
            kvT[g] = am.T[:GR, :].astype(BF)
            zb[g] = jnp.broadcast_to(a[:, GR:GR + 1], (2 * GR, TS))
        for c in range(NC):
            cg(c).wait()
            cu(c).wait()
            cd(c).wait()
        prep_l(0)

    def ffn(c, carry):
        def act(g, u, dh):
            g2 = g * g
            th = jnp.tanh(g * (GELU_C0 + (GELU_C0 * GELU_C1) * g2))
            hp = 0.5 * th + 0.5
            ge = g * hp
            dge = hp + (g * (1.0 - th * th)) * (0.5 * GELU_C0 + (1.5 * GELU_C0 * GELU_C1) * g2)
            return ge * u, (dh * u) * dge, dh * ge

        def s1(t):
            gu1, gu2 = _kt_dot(la[:256, :], lb[:256, :], ly[:256, :], xnT[t])
            dh1, dh2 = _kt_dot(la[256:, :], lb[256:, :], ly[256:, :], dyT[t])
            for n in range(2):
                for i in range(128 // RS):
                    rs = slice(i * RS, (i + 1) * RS)
                    ru = slice(128 + i * RS, 128 + (i + 1) * RS)
                    blk = []
                    for gu, dh in ((gu1, dh1), (gu2, dh2)):
                        for k in range(2):
                            cs = slice(k * TS + n * 128, k * TS + (n + 1) * 128)
                            blk.append(act(gu[rs, cs], gu[ru, cs], dh[rs, cs]))
                    for j in range(3):
                        for r, z in enumerate(_c_list(*[b[j] for b in blk])):
                            if j == 0:
                                ch[r, 2 * t + n, rs] = z
                            else:
                                cgu[r, 2 * t + n, rs if j == 1 else ru] = z

        ag = _a_list(wgu[c, :, :FC])
        au = _a_list(wgu[c, :, FC:])
        agu = [jnp.concatenate([p, q], axis=1) for p, q in zip(ag, au)]
        ad = _a_list(wdT[c])

        def s2(t):
            qgu, qd = [], []
            for r in range(7):
                h = jnp.concatenate([ch[r, 2 * t + n] for n in range(4)], axis=1)
                dgu = jnp.concatenate([cgu[r, 2 * t + n] for n in range(4)], axis=1)
                po = _nn(ad[r], h)
                pout[t, r] += po[:, :TS]
                pout[t + 1, r] += po[:, TS:]
                px = _nn(agu[r], dgu)
                pdx[t, r] += px[:, :TS]
                pdx[t + 1, r] += px[:, TS:]
                xb = jnp.concatenate([_b_get(bx, xnT, t, r), _b_get(bx, xnT, t + 1, r)], axis=1)
                yb = jnp.concatenate([_b_get(bdy, dyT, t, r), _b_get(bdy, dyT, t + 1, r)], axis=1)
                qgu.append(_nt(xb, dgu))
                qd.append(_nt(yb, h))
            return qgu, qd

        for t in range(NT):
            s1(t)
        prep_l(jnp.minimum(c + 1, NC - 1))
        qgu0, qd0 = s2(0)
        qgu1, qd1 = s2(2)
        qgu = [p + q for p, q in zip(qgu0, qgu1)]
        qd = [p + q for p, q in zip(qd0, qd1)]
        dwgu_o[c, :, :FC] = _q_combine([q[:, :128] for q in qgu]).astype(BF)
        dwgu_o[c, :, FC:] = _q_combine([q[:, 128:] for q in qgu]).astype(BF)
        dwd_o[c] = _q_combine(qd).astype(BF)
        o_g(c).start()
        o_u(c).start()
        o_d(c).start()
        return carry

    with jax.named_scope("ffn"):
        lax.fori_loop(0, NC, ffn, 0)

    def phase_b(t, carry):
        subs = [slice(s * TS, (s + 1) * TS) for s in range(T // TS)]
        os_, dps = [], []
        for sl in subs:
            pq = _nn(wpqT[...], xnT[t, :, sl])
            og, dpg = [], []
            for g in range(NG):
                ep, em, rp, rm = _softmax_pm(pq[g * GR:(g + 1) * GR])
                zp = zb[g, :GR, :].reshape(14, 8, TS)
                zm = zb[g, GR:, :].reshape(14, 8, TS)
                denp = _fold(ep * zp, jnp.sum) * rp
                denm = _fold(em * zm, jnp.sum) * rm
                den = denp + denm + DEN_EPS
                rden = 1.0 / den
                php = ep * (rp * rden)[None]
                phm = em * (rm * rden)[None]
                ph = jnp.concatenate([php.reshape(GR, TS).astype(BF), phm.reshape(GR, TS).astype(BF)], axis=0)
                do_g = doT[t, g * GR:(g + 1) * GR, sl]
                dd = _nn(kvb[g], do_g)
                og.append(_nn(kvT[g], ph).astype(BF))
                dp_ = dd[:GR].reshape(14, 8, TS)
                dm_ = dd[GR:].reshape(14, 8, TS)
                ap = _fold(php * dp_, jnp.sum)
                am = _fold(phm * dm_, jnp.sum)
                cc = ap + am
                tp = den * ap - cc * denp
                tm = den * am - cc * denm
                dpq = php * (dp_ - cc[None] * zp - tp[None]) - phm * (dm_ - cc[None] * zm - tm[None])
                dpg.append(dpq.reshape(GR, TS).astype(BF))
                cblk = jnp.concatenate([-cc, jnp.zeros((8, TS), F32)], axis=0).astype(BF)
                dkv[g] += _nt(ph, jnp.concatenate([do_g, cblk], axis=0))
            os_.append(jnp.concatenate(og, axis=0))
            dps.append(jnp.concatenate(dpg, axis=0))
        o = jnp.concatenate(os_, axis=1)
        dp = jnp.concatenate(dps, axis=1)
        out_o[t] = (xT[t].astype(F32) + _p_combine(pout, t) + _nn(woT[...], o)).astype(BF)
        dwo_acc[...] += _nt(o, dyT[t])
        gqT[...] += _nt(dp, xnT[t])
        dxT[t] = _p_combine(pdx, t) + _nn(wpq[...], dp)
        o_out(t).start()
        return carry

    with jax.named_scope("phaseB"):
        lax.fori_loop(0, NT, phase_b, 0)

    with jax.named_scope("midB"):
        keep_dkv = same_head | (col == row_j + GR)
        for g in range(NG):
            a = jnp.where(keep_dkv, dkv[g], 0.0)
            dkvb[g] = a.astype(BF)
            dkvT[g] = a.T[:GR, :].astype(BF)
        dwo_o[...] = dwo_acc[...].astype(BF)
        o_wo.start()

    def phase_c(t, carry):
        subs = [slice(s * TS, (s + 1) * TS) for s in range(T // TS)]
        sts = []
        for sl in subs:
            dvs, dps = [], []
            for g in range(NG):
                ph = phik[t, g * 2 * GR:(g + 1) * 2 * GR, sl]
                dphi = _nn(dkvb[g], vaug[t, g * 128:(g + 1) * 128, sl])
                dvs.append(_nn(dkvT[g], ph).astype(BF))
                phf = ph.astype(F32)
                php = phf[:GR].reshape(14, 8, TS)
                phm = phf[GR:].reshape(14, 8, TS)
                wp = php * dphi[:GR].reshape(14, 8, TS)
                wm = phm * dphi[GR:].reshape(14, 8, TS)
                tp = _fold(wp, jnp.sum)
                tm = _fold(wm, jnp.sum)
                dpk = (wp - wm) - (php * tp[None] - phm * tm[None])
                dps.append(dpk.reshape(GR, TS).astype(BF))
            sts.append(jnp.concatenate(dvs + dps, axis=0))
        st = jnp.concatenate(sts, axis=1)
        dxn = dxT[t] + _nn(wc[...], st)
        gvk[...] += _nt(xnT[t], st)
        xn = xnT[t].astype(F32)
        m1 = jnp.sum(dxn, axis=0, keepdims=True) * (1.0 / D)
        m2 = jnp.sum(dxn * xn, axis=0, keepdims=True) * (1.0 / D)
        dx = dyT[t].astype(F32) + rstd[t, 0:1, :] * (dxn - m1 - xn * m2)
        dx_o[t] = dx.astype(BF)
        o_dx(t).start()
        return carry

    with jax.named_scope("phaseC"):
        lax.fori_loop(0, NT, phase_c, 0)

    with jax.named_scope("tail"):
        gkT = gvk[:, 384:].astype(BF).T
        dbs = []
        for g in range(NG):
            gq = gqT[g * GR:(g + 1) * GR, :].astype(BF)
            gk = gkT[64 + g * GR:64 + (g + 1) * GR, :]
            bdg = bd[g * GR:(g + 1) * GR, :]
            dwqkT[g * GR:(g + 1) * GR, :] = _nn(bdg, gq).astype(BF)
            dwqkT[D + g * GR:D + (g + 1) * GR, :] = _nn(bdg, gk).astype(BF)
            dbs.append(_nt(wT[g * GR:(g + 1) * GR, :], gq) + _nt(wT[D + g * GR:D + (g + 1) * GR, :], gk))
        dwqkv_o[:, :2 * D] = dwqkT[...].T
        dwqkv_o[:, 2 * D:] = gvk[:, :D].astype(BF)
        o_wqkv.start()
        db = jnp.concatenate(dbs, axis=0)
        keep2 = (_div28(_iota((D, GR), 0)) & 3) == (_iota((D, GR), 1) & 3)
        db = jnp.where(keep2, db, 0.0).astype(BF)
        e_t = ((_iota((GR, DH), 0) >> 2) == _iota((GR, DH), 1)).astype(F32).astype(BF)
        db = _nn(db, e_t).astype(BF)
        r_i = _iota((D, D), 0)
        perm_t = (_iota((D, D), 1) == (r_i & 15) * DH + (r_i >> 4)).astype(F32).astype(BF)
        dwphi_o[...] = _nn(perm_t, db).astype(BF).reshape(DH, H, DH)
        o_wphi.start()

        for t in range(NT):
            o_out(t).wait()
            o_dx(t).wait()
        for c in range(NC):
            o_g(c).wait()
            o_u(c).wait()
            o_d(c).wait()
        o_wo.wait()
        o_wqkv.wait()
        o_wphi.wait()


@jax.jit
def pallas_parallel_sum__linear_kernel_hedgehog__glu_gated_geglu__prompt_kernel(
    A_x: jax.Array,
    A_wqkv: jax.Array,
    A_w_phi: jax.Array,
    A_wo: jax.Array,
    B_x: jax.Array,
    B_w_gate: jax.Array,
    B_w_up: jax.Array,
    B_w_down: jax.Array,
    grad_out: jax.Array,
):
    del B_x
    V = pltpu.VMEM
    dma = pltpu.SemaphoreType.DMA
    scratch = [
        V((NT, D, T), BF), V((NT, D, T), BF), V((D, 3 * D), BF), V((DH, H, DH), BF), V((D, D), BF),
        V((NC, D, 2 * FC), BF), V((NC, D, FC), BF),
        V((NT, D, T), BF), V((NT, 8, T), F32), V((NT, D, T), F32), V((NT, D, T), BF),
        V((NT, 2 * D, T), BF), V((NT, NG * 128, T), BF),
        V((3 * D, D), BF), V((D, D), BF), V((2 * D, D), BF), V((D, D), BF), V((D, D), BF), V((D, 2 * D), BF),
        V((D, GR), BF),
        V((NG, 2 * GR, 128), F32), V((NG, 2 * GR, GR), BF), V((NG, GR, 2 * GR), BF), V((NG, 2 * GR, TS), F32),
        V((NG, 2 * GR, 128), F32), V((NG, 2 * GR, 128), BF), V((NG, GR, 2 * GR), BF),
        V((D, D), F32), V((D, 2 * D), F32), V((D, D), F32),
        V((NT, 5, DD, TS), BF), V((NT, 5, DD, TS), BF), V((NT, 7, DD, TS), F32), V((NT, 7, DD, TS), F32),
        V((3 * 128, 384), BF), V((3 * 128, 384), BF), V((3 * 128, 128), BF),
        V((7, 2 * NT, 128, 128), BF), V((7, 2 * NT, 256, 128), BF),
        V((NT, D, T), BF), V((NT, D, T), BF), V((D, 3 * D), BF), V((DH, H, DH), BF), V((D, D), BF),
        V((NC, D, 2 * FC), BF), V((NC, D, FC), BF), V((2 * D, D), BF),
        dma((NT,)), dma((NT,)), dma((3,)), dma((NC,)), dma((NC,)), dma((NC,)),
        dma((NT,)), dma((NT,)), dma((3,)), dma((NC,)), dma((NC,)), dma((NC,)),
    ]
    sds = jax.ShapeDtypeStruct
    out_shape = (
        sds((D, S), BF), sds((D, S), BF), sds((D, 3 * D), BF), sds((DH, H, DH), BF), sds((D, D), BF),
        sds((D, F), BF), sds((D, F), BF), sds((D, F), BF),
    )
    hbm = pl.BlockSpec(memory_space=pl.ANY)
    outT, dxT, dwqkv, dwphi, dwo, dwg, dwu, dwdT = pl.pallas_call(
        _kernel,
        out_shape=out_shape,
        in_specs=[hbm] * 8,
        out_specs=(hbm,) * 8,
        scratch_shapes=scratch,
        compiler_params=pltpu.CompilerParams(vmem_limit_bytes=100 * 2 ** 20),
        name="hedgehog_geglu_fwdbwd",
    )(A_x.reshape(S, D).T, A_wqkv, A_w_phi.transpose(1, 0, 2), A_wo, B_w_gate, B_w_up, B_w_down.T,
      grad_out.reshape(S, D).T)
    return (outT.T.reshape(1, S, D), dxT.T.reshape(1, S, D), dwqkv, dwphi.transpose(1, 0, 2), dwo,
            dwg, dwu, dwdT.T)
```

```python
import jax
import jax.numpy as jnp
import jax.experimental.pallas as pl
import jax.experimental.pallas.tpu as pltpu
from jax import lax

S = 2048
D = 448
F = 1792
H = 16
DH = 28
NG = 4
GR = 112
NP = 8
PR = 56
T = 512
NT = S // T
TS = 256
FC = 256
NC = F // FC
RS = 32
NW = 128
NLAST = 3
DQ = D // 4
DD = D // 2
BF = jnp.bfloat16
F32 = jnp.float32
LN_EPS = 1e-5
DEN_EPS = 1e-6
GELU_C0 = 0.7978845608028654
GELU_C1 = 0.044715


def _nn(a, b):
    return lax.dot_general(a, b, (((1,), (0,)), ((), ())), preferred_element_type=F32)


def _nt(a, b):
    return lax.dot_general(a, b, (((1,), (1,)), ((), ())), preferred_element_type=F32)


def _iota(shape, dim):
    return lax.broadcasted_iota(jnp.int32, shape, dim)


def _div28(r):
    return (r * 9363) >> 18


def _fold(x, op):
    f = {jnp.max: jnp.maximum, jnp.min: jnp.minimum, jnp.sum: jnp.add}[op]
    r = op(x, axis=0)
    r = f(r, pltpu.roll(r, 4, 0))
    return f(r, pltpu.roll(r, 2, 0))


def _softmax_pm(p):
    n = p.shape[-1]
    p3 = p.reshape(7, 8, n)
    mx = _fold(p3, jnp.max)
    mn = _fold(p3, jnp.min)
    ep = jnp.exp(p3 - mx[None])
    em = jnp.exp(mn[None] - p3)
    rp = 1.0 / _fold(ep, jnp.sum)
    rm = 1.0 / _fold(em, jnp.sum)
    return ep, em, rp, rm


A_T = [{(0, 0): 1, (1, 1): 1}, {(0, 1): 1, (1, 1): 1}, {(0, 0): 1}, {(1, 1): 1}, {(0, 0): 1, (1, 0): 1},
       {(0, 1): 1, (0, 0): -1}, {(1, 0): 1, (1, 1): -1}]
B_T = [{(0, 0): 1, (1, 1): 1}, {(0, 0): 1}, {(0, 1): 1, (1, 1): -1}, {(1, 0): 1, (0, 0): -1}, {(1, 1): 1},
       {(0, 0): 1, (0, 1): 1}, {(1, 0): 1, (1, 1): 1}]
C_T = [{(0, 0): 1, (1, 1): 1}, {(1, 0): 1, (1, 1): -1}, {(0, 1): 1, (1, 1): 1}, {(0, 0): 1, (1, 0): 1},
       {(0, 1): 1, (0, 0): -1}, {(1, 1): 1}, {(0, 0): 1}]


def _acc(terms):
    terms = sorted(terms, key=lambda p: -p[0])
    z = terms[0][1] if terms[0][0] > 0 else -terms[0][1]
    for sg, v in terms[1:]:
        z = z + v if sg > 0 else z - v
    return z


def _lin(tab, r, get):
    return _acc([(sg, get(i, j)) for (i, j), sg in tab[r].items()])


def _lin2(tab, r1, r2, get):
    terms = [(s1 * s2, get(2 * i1 + i2, 2 * j1 + j2))
             for (i1, j1), s1 in tab[r1].items() for (i2, j2), s2 in tab[r2].items()]
    if len(terms) < 4:
        return _acc(terms)
    return _acc([(1, _acc([terms[0], terms[3]])), terms[1], terms[2]])


def _comb(tab, i, j, get):
    return _acc([(tab[r][(i, j)], get(r)) for r in range(7) if (i, j) in tab[r]])


def _swap64(a, b):
    a = pltpu.bitcast(a, jnp.uint32)
    b = pltpu.bitcast(b, jnp.uint32)
    lo = _iota(a.shape, 1) < 64
    p = jnp.where(lo, a, pltpu.roll(b, 64, 1))
    q = jnp.where(lo, pltpu.roll(a, 64, 1), b)
    return pltpu.bitcast(p, BF), pltpu.bitcast(q, BF)


def _b_sums(x):
    b11, b12, b21, b22 = x[:DD, :TS], x[:DD, TS:], x[DD:, :TS], x[DD:, TS:]
    return [b11 + b22, b12 - b22, b21 - b11, b11 + b12, b21 + b22]


def _b_get(bs, full, t, r):
    if r == 1:
        return full[t, :DD, :TS]
    if r == 4:
        return full[t, DD:, TS:]
    return bs[t, {0: 0, 2: 1, 3: 2, 5: 3, 6: 4}[r]]


def _a_list(w):
    w11, w12, w21, w22 = w[:DD, :128], w[:DD, 128:], w[DD:, :128], w[DD:, 128:]
    f = lambda z: z.astype(F32)
    return [(f(w11) + f(w22)).astype(BF), (f(w12) + f(w22)).astype(BF), w11, w22,
            (f(w11) + f(w21)).astype(BF), (f(w12) - f(w11)).astype(BF), (f(w21) - f(w22)).astype(BF)]


def _c_list(c11, c12, c21, c22):
    return [z.astype(BF) for z in (c11 + c22, c21 - c22, c12 + c22, c11 + c21, c12 - c11, c22, c11)]


def _p_combine(p, t):
    top = jnp.concatenate([p[t, 0] + p[t, 1] - p[t, 3] + p[t, 5], p[t, 2] + p[t, 5]], axis=1)
    bot = jnp.concatenate([p[t, 3] + p[t, 6], p[t, 0] - p[t, 2] + p[t, 4] + p[t, 6]], axis=1)
    return jnp.concatenate([top, bot], axis=0)


def _q_combine(q):
    top = jnp.concatenate([q[0] + q[2] + q[4] - q[5], q[1] + q[5]], axis=1)
    bot = jnp.concatenate([q[4] + q[6], q[0] + q[1] + q[3] - q[6]], axis=1)
    return jnp.concatenate([top, bot], axis=0)


def _kt_rows(w):
    w1, w2 = w[:, :128], w[:, 128:]
    dz = (w1[256:384].astype(F32) - w2[256:384].astype(F32))
    a = jnp.concatenate([w1[:256], dz[64:].astype(BF), w1[384:]], axis=0)
    b = jnp.concatenate([w2[:256], (-dz[:64]).astype(BF), w2[384:]], axis=0)
    y = jnp.concatenate([w1[256:320], w2[320:384]], axis=0)
    return a.T, b.T, y.T


def _kt_form(w1, w2):
    dz = w1[:, 256:384] - w2[:, 256:384]
    y = jnp.concatenate([w1[:, 256:320], w2[:, 320:384]], axis=1)
    a = jnp.concatenate([dz[:, 64:], w1[:, 384:]], axis=1)
    b = jnp.concatenate([-dz[:, :64], w2[:, 384:]], axis=1)
    return [z.astype(BF) for z in (y, a, b)]


def _kt(m01, y, a, b, x):
    m = y.shape[0]
    yy = _nn(y, x[256:384])
    a2 = _nn(a, x[320:])
    b2 = _nn(b, jnp.concatenate([x[256:320], x[384:]], axis=0))
    mm = _nn(m01, x[:256])
    return (yy + a2) + mm[:m], (yy + b2) + mm[m:]


def _feat(col):
    p = (col >= PR).astype(jnp.int32)
    rem = col - p * PR
    return rem >> 1, 2 * p + (rem & 1)


def _kernel(xT_h, wqkv_h, wphi_h, wo_h, wg_h, wu_h, wdT_h, dyT_h,
            out_h, dx_h, dwqkv_h, dwphi_h, dwo_h, dwg_h, dwu_h, dwdT_h,
            xT, dyT, wqkv, wphi, wo, w3,
            xnT, xn0, rstd, dxT, doT, phik, vaug, o_s, dp_s, st_s,
            wT, woT, wa, wa3, wpqT, wq3, wo3, wpq, wc, wcT, bd,
            kv, kvb, kvT, zb, dkv, dkvb, dkvT, gqT, gvk, dwo_acc,
            bx, bdy, pout, pdx, la, lb, ly, hr0, hr1, gur,
            out_o, dx_o, dwqkv_o, dwphi_o, dwo_o, dwgu_o, dwd_o, dwqkT,
            s_x, s_dy, s_w, s_f, so_out, so_dx, so_w, so_g, so_u, so_d):
    cp = pltpu.make_async_copy

    def tok(t):
        return pl.ds(pl.multiple_of(t * T, T), T)

    def fch(c):
        return pl.ds(pl.multiple_of(c * FC, FC), FC)

    def cx(t):
        return cp(xT_h.at[:, tok(t)], xT.at[t], s_x.at[t])

    def cdy(t):
        return cp(dyT_h.at[:, tok(t)], dyT.at[t], s_dy.at[t])

    def cf(c, i):
        return cp((wg_h, wu_h, wdT_h)[i].at[:, fch(c)], w3.at[3 * c + i], s_f.at[3 * c + i])

    c_wo = cp(wo_h, wo, s_w.at[0])
    c_wphi = cp(wphi_h, wphi, s_w.at[1])
    c_wqkv = cp(wqkv_h, wqkv, s_w.at[2])

    def o_out(t):
        return cp(out_o.at[t], out_h.at[:, tok(t)], so_out.at[t])

    def o_dx(t):
        return cp(dx_o.at[t], dx_h.at[:, tok(t)], so_dx.at[t])

    def o_g(c):
        return cp(dwgu_o.at[c, :, pl.ds(0, FC)], dwg_h.at[:, fch(c)], so_g.at[c])

    def o_u(c):
        return cp(dwgu_o.at[c, :, pl.ds(FC, FC)], dwu_h.at[:, fch(c)], so_u.at[c])

    def o_d(c):
        return cp(dwd_o.at[c], dwdT_h.at[:, fch(c)], so_d.at[c])

    o_wqkv = cp(dwqkv_o, dwqkv_h, so_w.at[0])
    o_wphi = cp(dwphi_o, dwphi_h, so_w.at[1])
    o_wo = cp(dwo_o, dwo_h, so_w.at[2])

    c_wphi.start()
    c_wo.start()
    for t in range(3):
        cdy(t).start()
    c_wqkv.start()
    cdy(3).start()
    cx(0).start()
    cx(1).start()
    cf(0, 0).start()
    cx(2).start()
    cf(0, 1).start()
    cx(3).start()
    cf(0, 2).start()
    for c in range(1, NC):
        for i in range(3):
            cf(c, i).start()

    lanes = [slice(j * 128, (j + 1) * 128) for j in range(4)]

    def do_tile(t):
        z8 = jnp.zeros((8, 128), F32)
        for s in range(2):
            for sl in lanes:
                r = _kt(wo[s * DD:(s + 1) * DD, :256], wo3[s, 0], wo3[s, 1], wo3[s, 2], dyT[t, :, sl])
                for k in range(2):
                    g = 2 * s + k
                    doT[t, g * 128:(g + 1) * 128, sl] = jnp.concatenate([r[k][:PR], z8, r[k][PR:], z8], axis=0).astype(BF)

    def dy_sums(t):
        for i, r in enumerate((0, 2, 3, 5, 6)):
            for m in range(2):
                get = lambda a, b: dyT[t, a * DD:(a + 1) * DD, lanes[2 * b + m]].astype(F32)
                bdy[t, i, :, lanes[m]] = _lin(B_T, r, get).astype(BF)

    def layer_norm(t, sl):
        x = xT[t, :, sl].astype(F32)
        mu = jnp.sum(x, axis=0, keepdims=True) * (1.0 / D)
        xc = x - mu
        var = jnp.sum(xc * xc, axis=0, keepdims=True) * (1.0 / D)
        rs = lax.rsqrt(var + LN_EPS)
        rstd[t, :, sl] = jnp.broadcast_to(rs, (8, 128))
        return (xc * rs).astype(BF)

    with jax.named_scope("head0"):
        w3[3 * NC] = jnp.zeros((D, FC), BF)
        kv[...] = jnp.zeros_like(kv)
        dkv[...] = jnp.zeros_like(dkv)
        gqT[...] = jnp.zeros_like(gqT)
        gvk[...] = jnp.zeros_like(gvk)
        dwo_acc[...] = jnp.zeros_like(dwo_acc)
        c_wphi.wait()
        pw = wphi[...].reshape(DH * H, DH)
        e_m = (_iota((DH, GR), 0) == _feat(_iota((DH, GR), 1))[0]).astype(F32).astype(BF)
        q_m = _nn(pw, e_m)
        keep = (_iota((D, GR), 0) & 3) == _feat(_iota((D, GR), 1))[1]
        q_m = jnp.where(keep, q_m, 0.0).astype(BF)
        r_i = _iota((D, D), 0)
        r_h = _div28(r_i)
        perm = (_iota((D, D), 1) == (r_i - r_h * DH) * H + r_h).astype(F32).astype(BF)
        bd[...] = _nn(perm, q_m).astype(BF)
        c_wo.wait()
        for s in range(2):
            w = wo[s * DD:(s + 1) * DD, :].astype(F32)
            for i, z in enumerate(_kt_form(w[:GR], w[GR:])):
                wo3[s, i] = z

    def head1(t, carry):
        cdy(t).wait()
        do_tile(t)
        dy_sums(jnp.minimum(t, NT - 1))
        return carry

    with jax.named_scope("head1"):
        lax.fori_loop(0, NT - 1, head1, 0)
    with jax.named_scope("head2"):
        c_wqkv.wait()
        cdy(3).wait()
        do_tile(3)
        wT[...] = wqkv[...].T
        cx(0).wait()
    with jax.named_scope("head3"):
        for g in range(NG):
            bdt = bd[g * GR:(g + 1) * GR, :].T
            pk = _nn(bdt, wT[D + g * GR:D + (g + 1) * GR, :])
            vf = wT[2 * D + g * GR:2 * D + (g + 1) * GR, :].astype(F32)
            w1 = jnp.concatenate([pk[:PR], vf[:PR]], axis=0)
            w2 = jnp.concatenate([pk[PR:], vf[PR:]], axis=0)
            wa[g * DD:(g + 1) * DD, :] = jnp.concatenate([w1, w2], axis=0).astype(BF)
            for i, z in enumerate(_kt_form(w1, w2)):
                wa3[g, i] = z
            wc[D + g * GR:D + (g + 1) * GR, :] = pk.astype(BF)
        xn0[...] = layer_norm(0, lanes[0])
        dy_sums(3)
        woT[...] = wo[...].T
        pqs = [_nn(bd[g * GR:(g + 1) * GR, :].T, wT[g * GR:(g + 1) * GR, :]) for g in range(NG)]
        for s in range(2):
            for i, z in enumerate(_kt_form(pqs[2 * s], pqs[2 * s + 1])):
                wq3[s, i] = z
        wpqT[...] = jnp.concatenate(pqs, axis=0).astype(BF)
        wc[:D, :] = wT[2 * D:, :]
        wpq[...] = wpqT[...].T
        wcT[...] = wc[...].T

    def prep_l(src, i):
        a, b, y = _kt_rows(w3[src])
        rows = pl.ds(i * 128, 128) if isinstance(i, int) else pl.ds(pl.multiple_of(i * 128, 128), 128)
        la[rows, :] = a
        lb[rows, :] = b
        ly[rows, :] = y

    def phase_a(t, carry):
        @pl.when(t < NT - 1)
        def _():
            cx(t + 1).wait()

        @pl.when(t > 0)
        def _():
            cp(wg_h.at[:, fch(0)], w3.at[t - 1], s_f.at[t - 1]).wait()

        ones = jnp.ones((8, 128), F32)
        xns = [xn0[...]] + [layer_norm(t, sl) for sl in lanes[1:]]
        for j, sl in enumerate(lanes):
            xnT[t, :, sl] = xns[j]
            for g in range(NG):
                r = _kt(wa[g * DD:(g + 1) * DD, :256], wa3[g, 0], wa3[g, 1], wa3[g, 2], xns[j])
                for k in range(2):
                    p = 2 * g + k
                    ep, em, rp, rm = _softmax_pm(r[k][:PR])
                    ph = jnp.concatenate([(ep * rp[None]).reshape(PR, 128), (em * rm[None]).reshape(PR, 128)], axis=0)
                    phik[t, p * GR:(p + 1) * GR, sl] = ph.astype(BF)
                    vaug[t, p * 64:(p + 1) * 64, sl] = jnp.concatenate([r[k][PR:], ones], axis=0).astype(BF)
        for p in range(NP):
            kv[p] += _nt(vaug[t, p * 64:(p + 1) * 64, :], phik[t, p * GR:(p + 1) * GR, :])
        xn0[...] = layer_norm(jnp.minimum(t + 1, NT - 1), lanes[0])
        for r1 in range(7):
            for r2 in range(7):
                get = lambda i, j: xns[j][i * DQ:(i + 1) * DQ].astype(F32)
                bx[7 * r1 + r2, t] = _lin2(B_T, r1, r2, get).astype(BF)
        prep_l(jnp.where(t == 0, 3 * NC, t - 1), jnp.maximum(t - 1, 0))
        return carry

    with jax.named_scope("phaseA"):
        lax.fori_loop(0, NT, phase_a, 0)

    row = _iota((64, GR), 0)
    col_j = _iota((64, GR), 1) & 1
    same_head = (row < PR) & ((row >= DH).astype(jnp.int32) == col_j)

    with jax.named_scope("midA"):
        for c in range(1, NC):
            for i in range(3):
                cf(c, i).wait()

    def ffn(c, carry):
        def act(g, u, dh):
            g2 = g * g
            th = jnp.tanh(g * (GELU_C0 + (GELU_C0 * GELU_C1) * g2))
            hp = 0.5 * th + 0.5
            ge = g * hp
            dge = hp + (g * (1.0 - th * th)) * (0.5 * GELU_C0 + (1.5 * GELU_C0 * GELU_C1) * g2)
            return ge * u, (dh * u) * dge, dh * ge

        def kt(rows, x):
            cat = lambda ref, cs: jnp.concatenate([ref[r, cs] for r in rows], axis=0)
            m01 = jnp.concatenate([cat(la, slice(0, 256)), cat(lb, slice(0, 256))], axis=0)
            return _kt(m01, cat(ly, slice(None)), cat(la, slice(256, 384)), cat(lb, slice(256, 384)), x)

        def s1(t, n, i):
            ls = slice(n * NW, (n + 1) * NW)
            rg, ru, rd = [slice(k * 128 + i * RS, k * 128 + (i + 1) * RS) for k in range(3)]
            dhs = kt([rd], dyT[t, :, ls])
            ugs = kt([ru, rg], xnT[t, :, ls])
            for k in range(2):
                h, dg, du = act(ugs[k][RS:], ugs[k][:RS], dhs[k])
                for m in range(NW // 128):
                    j = 4 * t + n * (NW // 128) + m + (c >> 3)
                    cs = slice(m * 128, (m + 1) * 128)
                    (hr0 if t < 2 else hr1)[j - 8 * (t // 2), k * 128 + i * RS:k * 128 + (i + 1) * RS] = h[:, cs]
                    for e in range(max(RS // 64, 1)):
                        w = min(RS, 64)
                        q, o = divmod(k * 128 + i * RS + e * 64, 64)
                        gur[j, q, o:o + w] = dg[e * 64:e * 64 + w, cs]
                        gur[j, q, 64 + o:64 + o + w] = du[e * 64:e * 64 + w, cs]

        for t in range(NT):
            for n in range(T // NW):
                for i in range(128 // RS):
                    s1(t, n, i)
        cn = jnp.minimum(c + 1, NC - 1)
        for i in range(3):
            prep_l(3 * cn + i, i)
        for p in (c, c + 1):
            a = kv[p]
            am = jnp.where(same_head, a, 0.0)
            kvT[p] = am.astype(BF)
            kvb[p] = am.T.astype(BF)
            zb[p] = jnp.broadcast_to(a.T[:, PR:PR + 1], (GR, 128))

        wq = _swap64(w3[3 * c, :, :128], w3[3 * c + 1, :, :128]) + _swap64(w3[3 * c, :, 128:], w3[3 * c + 1, :, 128:])
        wq = [w.astype(F32) for w in wq]
        ad = _a_list(w3[3 * c + 2])

        def hsum(t, r):
            ref = hr0 if t == 0 else hr1
            return jnp.concatenate([_lin(C_T, r, lambda k, j: ref[4 * e + 2 * j + m, k * 128:(k + 1) * 128])
                                    for e in range(2) for m in range(2)], axis=1).astype(BF)

        def hp(t, r, h):
            po = _nn(ad[r], h)
            pout[t, r] = jnp.where(c > 0, pout[t, r], 0.0) + po[:, :TS]
            pout[t + 1, r] = jnp.where(c > 0, pout[t + 1, r], 0.0) + po[:, TS:]

        def hq(t, r, h):
            return _nt(jnp.concatenate([_b_get(bdy, dyT, t, r), _b_get(bdy, dyT, t + 1, r)], axis=1), h)

        qd0 = []
        for r in range(7):
            h = hsum(0, r)
            hp(0, r, h)
            qd0.append(hq(0, r, h))
        q1, qd, hs = [], [], []
        for r1 in range(7):
            q2 = []
            for r2 in range(7):
                r = 7 * r1 + r2
                a = _lin2(A_T, r1, r2, lambda i, k: wq[k][i * DQ:(i + 1) * DQ]).astype(BF)
                cc = jnp.concatenate([_lin2(C_T, r1, r2, lambda k, j: gur[4 * t + j, k]) for t in range(NT)], axis=1).astype(BF)
                px = _nn(a, cc)
                for t in range(NT):
                    pdx[t, r] = jnp.where(c > 0, pdx[t, r], 0.0) + px[:, t * 128:(t + 1) * 128]
                q2.append(_nt(jnp.concatenate([bx[r, t] for t in range(NT)], axis=1), cc))
            q1.append({(i, k): _comb(A_T, i, k, lambda r: q2[r]) for i in range(2) for k in range(2)})
            h = hsum(2, r1)
            qd.append(qd0[r1] + hq(2, r1, h))
            if r1 < 7 - NLAST:
                hp(2, r1, h)
            else:
                hs.append((r1, h))
        for k1 in range(2):
            cols = [jnp.concatenate([_comb(A_T, i1, k1, lambda r: q1[r][(i2, k2)])
                                     for i1 in range(2) for i2 in range(2)], axis=0).astype(BF) for k2 in range(2)]
            g_, u_ = _swap64(*cols)
            dwgu_o[c, :, k1 * 128:(k1 + 1) * 128] = g_
            dwgu_o[c, :, FC + k1 * 128:FC + (k1 + 1) * 128] = u_
        dwd_o[c] = _q_combine(qd).astype(BF)
        for r1, h in hs:
            hp(2, r1, h)
        o_g(c).start()
        o_u(c).start()
        o_d(c).start()
        return carry

    with jax.named_scope("ffn"):
        lax.fori_loop(0, NC, ffn, 0)

    def phase_b(t, carry):
        def stage1(s, sl):
            return _kt(wpqT[s * DD:(s + 1) * DD, :256], wq3[s, 0], wq3[s, 1], wq3[s, 2], xnT[t, :, sl])

        def stage2(g, sl, pq):
            og, dpg = [], []
            for k in range(2):
                p = 2 * g + k
                do_p = doT[t, p * 64:(p + 1) * 64, sl]
                dd = _nn(kvb[p], do_p)
                ep, em, rp, rm = _softmax_pm(pq[k * PR:(k + 1) * PR])
                zp = zb[p, :PR, :].reshape(7, 8, 128)
                zm = zb[p, PR:, :].reshape(7, 8, 128)
                denp = _fold(ep * zp, jnp.sum) * rp
                denm = _fold(em * zm, jnp.sum) * rm
                den = denp + denm + DEN_EPS
                rden = 1.0 / den
                php = ep * (rp * rden)[None]
                phm = em * (rm * rden)[None]
                ph = jnp.concatenate([php.reshape(PR, 128), phm.reshape(PR, 128)], axis=0).astype(BF)
                og.append(_nn(kvT[p], ph)[:PR])
                dp_ = dd[:PR].reshape(7, 8, 128)
                dm_ = dd[PR:].reshape(7, 8, 128)
                ap = _fold(php * dp_, jnp.sum)
                am = _fold(phm * dm_, jnp.sum)
                cc = ap + am
                tp = den * ap - cc * denp
                tm = den * am - cc * denm
                dpq = php * (dp_ - cc[None] * zp - tp[None]) - phm * (dm_ - cc[None] * zm - tm[None])
                dpg.append(dpq.reshape(PR, 128))
                last = jnp.concatenate([do_p[48:].astype(F32)[:8], -cc], axis=0).astype(BF)
                dkv[p] += _nt(jnp.concatenate([do_p[:48], last], axis=0), ph)
            o_s[g * GR:(g + 1) * GR, sl] = jnp.concatenate(og, axis=0).astype(BF)
            dp_s[g * GR:(g + 1) * GR, sl] = jnp.concatenate(dpg, axis=0).astype(BF)

        items = [(s, sl) for s in range(2) for sl in lanes]
        nxt = stage1(*items[0])
        for i, (s, sl) in enumerate(items):
            cur = nxt
            if i + 1 < len(items):
                nxt = stage1(*items[i + 1])
            for k in range(2):
                stage2(2 * s + k, sl, cur[k])
        o = o_s[...]
        dp = dp_s[...]
        out_o[t] = (xT[t].astype(F32) + _p_combine(pout, t) + _nn(woT[...], o)).astype(BF)
        dwo_acc[...] += _nt(o, dyT[t])
        gqT[...] += _nt(dp, xnT[t])
        p1 = [{(i, j): _comb(B_T, i, j, lambda r: pdx[t, 7 * r1 + r]) for i in range(2) for j in range(2)} for r1 in range(7)]
        pc = jnp.concatenate([jnp.concatenate([_comb(B_T, i1, j1, lambda r: p1[r][(i2, j2)])
                                               for j1 in range(2) for j2 in range(2)], axis=1)
                              for i1 in range(2) for i2 in range(2)], axis=0)
        dxT[t] = pc + _nn(wpq[...], dp)
        o_out(t).start()
        return carry

    with jax.named_scope("phaseB"):
        lax.fori_loop(0, NT, phase_b, 0)

    with jax.named_scope("midB"):
        keep_dkv = same_head | (row == col_j + PR)
        for p in range(NP):
            a = jnp.where(keep_dkv, dkv[p], 0.0)
            dkvT[p] = a.astype(BF)
            dkvb[p] = a.T.astype(BF)
        dwo_o[...] = dwo_acc[...].astype(BF)
        o_wo.start()

    def phase_c(t, carry):
        for g in range(NG):
            for sl in lanes:
                dvs, dps = [], []
                for k in range(2):
                    p = 2 * g + k
                    ph = phik[t, p * GR:(p + 1) * GR, sl]
                    dphi = _nn(dkvb[p], vaug[t, p * 64:(p + 1) * 64, sl])
                    dvs.append(_nn(dkvT[p], ph)[:PR])
                    phf = ph.astype(F32)
                    php = phf[:PR].reshape(7, 8, 128)
                    phm = phf[PR:].reshape(7, 8, 128)
                    wp = php * dphi[:PR].reshape(7, 8, 128)
                    wm = phm * dphi[PR:].reshape(7, 8, 128)
                    tp = _fold(wp, jnp.sum)
                    tm = _fold(wm, jnp.sum)
                    dpk = (wp - wm) - (php * tp[None] - phm * tm[None])
                    dps.append(dpk.reshape(PR, 128))
                st_s[g * GR:(g + 1) * GR, sl] = jnp.concatenate(dvs, axis=0).astype(BF)
                st_s[D + g * GR:D + (g + 1) * GR, sl] = jnp.concatenate(dps, axis=0).astype(BF)
        st = st_s[...]
        dxn = dxT[t] + _nn(wcT[...], st)
        gvk[...] += _nt(xnT[t], st)
        xn = xnT[t].astype(F32)
        m1 = jnp.sum(dxn, axis=0, keepdims=True) * (1.0 / D)
        m2 = jnp.sum(dxn * xn, axis=0, keepdims=True) * (1.0 / D)
        dx = dyT[t].astype(F32) + rstd[t, 0:1, :] * (dxn - m1 - xn * m2)
        dx_o[t] = dx.astype(BF)
        o_dx(t).start()
        return carry

    with jax.named_scope("phaseC"):
        lax.fori_loop(0, NT, phase_c, 0)

    with jax.named_scope("tail"):
        gkT = gvk[:, 384:].astype(BF).T
        dbs = []
        for g in range(NG):
            gq = gqT[g * GR:(g + 1) * GR, :].astype(BF)
            gk = gkT[64 + g * GR:64 + (g + 1) * GR, :]
            bdg = bd[g * GR:(g + 1) * GR, :]
            dwqkT[g * GR:(g + 1) * GR, :] = _nn(bdg, gq).astype(BF)
            dwqkT[D + g * GR:D + (g + 1) * GR, :] = _nn(bdg, gk).astype(BF)
            dbs.append(_nt(wT[g * GR:(g + 1) * GR, :], gq) + _nt(wT[D + g * GR:D + (g + 1) * GR, :], gk))
        dwqkv_o[:, :2 * D] = dwqkT[...].T
        dwqkv_o[:, 2 * D:] = gvk[:, :D].astype(BF)
        o_wqkv.start()
        db = jnp.concatenate(dbs, axis=0)
        keep2 = (_div28(_iota((D, GR), 0)) & 3) == _feat(_iota((D, GR), 1))[1]
        db = jnp.where(keep2, db, 0.0).astype(BF)
        e_t = (_feat(_iota((GR, DH), 0))[0] == _iota((GR, DH), 1)).astype(F32).astype(BF)
        db = _nn(db, e_t).astype(BF)
        r_i = _iota((D, D), 0)
        perm_t = (_iota((D, D), 1) == (r_i & 15) * DH + (r_i >> 4)).astype(F32).astype(BF)
        dwphi_o[...] = _nn(perm_t, db).astype(BF).reshape(DH, H, DH)
        o_wphi.start()

        for t in range(NT):
            o_out(t).wait()
            o_dx(t).wait()
        for c in range(NC):
            o_g(c).wait()
            o_u(c).wait()
            o_d(c).wait()
        o_wo.wait()
        o_wqkv.wait()
        o_wphi.wait()


@jax.jit
def pallas_parallel_sum__linear_kernel_hedgehog__glu_gated_geglu__prompt_kernel(
    A_x: jax.Array,
    A_wqkv: jax.Array,
    A_w_phi: jax.Array,
    A_wo: jax.Array,
    B_x: jax.Array,
    B_w_gate: jax.Array,
    B_w_up: jax.Array,
    B_w_down: jax.Array,
    grad_out: jax.Array,
):
    del B_x
    V = pltpu.VMEM
    dma = pltpu.SemaphoreType.DMA
    scratch = [
        V((NT, D, T), BF), V((NT, D, T), BF), V((D, 3 * D), BF), V((DH, H, DH), BF), V((D, D), BF),
        V((3 * NC + 1, D, FC), BF),
        V((NT, D, T), BF), V((D, 128), BF), V((NT, 8, T), F32), V((NT, D, T), F32), V((NT, NP * 64, T), BF),
        V((NT, 2 * D, T), BF), V((NT, NP * 64, T), BF), V((D, T), BF), V((D, T), BF), V((2 * D, T), BF),
        V((3 * D, D), BF), V((D, D), BF), V((2 * D, D), BF), V((NG, 3, GR, 128), BF), V((D, D), BF),
        V((2, 3, GR, 128), BF), V((2, 3, GR, 128), BF), V((D, D), BF), V((2 * D, D), BF), V((D, 2 * D), BF),
        V((D, GR), BF),
        V((NP, 64, GR), F32), V((NP, GR, 64), BF), V((NP, 64, GR), BF), V((NP, GR, 128), F32),
        V((NP, 64, GR), F32), V((NP, GR, 64), BF), V((NP, 64, GR), BF),
        V((D, D), F32), V((D, 2 * D), F32), V((D, D), F32),
        V((49, NT, DQ, 128), BF), V((NT, 5, DD, TS), BF), V((NT, 7, DD, TS), F32), V((NT, 49, DQ, 128), F32),
        V((3 * 128, 384), BF), V((3 * 128, 384), BF), V((3 * 128, 128), BF),
        V((2 * NT, FC, 128), F32), V((2 * NT, FC, 128), F32), V((4 * NT, 4, 128, 128), F32),
        V((NT, D, T), BF), V((NT, D, T), BF), V((D, 3 * D), BF), V((DH, H, DH), BF), V((D, D), BF),
        V((NC, D, 2 * FC), BF), V((NC, D, FC), BF), V((2 * D, D), BF),
        dma((NT,)), dma((NT,)), dma((3,)), dma((3 * NC,)),
        dma((NT,)), dma((NT,)), dma((3,)), dma((NC,)), dma((NC,)), dma((NC,)),
    ]
    sds = jax.ShapeDtypeStruct
    out_shape = (
        sds((D, S), BF), sds((D, S), BF), sds((D, 3 * D), BF), sds((DH, H, DH), BF), sds((D, D), BF),
        sds((D, F), BF), sds((D, F), BF), sds((D, F), BF),
    )
    hbm = pl.BlockSpec(memory_space=pl.ANY)
    outT, dxT, dwqkv, dwphi, dwo, dwg, dwu, dwdT = pl.pallas_call(
        _kernel,
        out_shape=out_shape,
        in_specs=[hbm] * 8,
        out_specs=(hbm,) * 8,
        scratch_shapes=scratch,
        compiler_params=pltpu.CompilerParams(vmem_limit_bytes=100 * 2 ** 20),
        name="hedgehog_geglu_fwdbwd",
    )(A_x.reshape(S, D).T, A_wqkv, A_w_phi.transpose(1, 0, 2), A_wo, B_w_gate, B_w_up, B_w_down.T,
      grad_out.reshape(S, D).T)
    return (outT.T.reshape(1, S, D), dxT.T.reshape(1, S, D), dwqkv, dwphi.transpose(1, 0, 2), dwo,
            dwg, dwu, dwdT.T)
```

```python
import jax
import jax.numpy as jnp
import jax.experimental.pallas as pl
import jax.experimental.pallas.tpu as pltpu
from jax import lax

S = 2048
D = 448
F = 1792
H = 16
DH = 28
NG = 4
GR = 112
NP = 8
PR = 56
T = 512
NT = S // T
TS = 256
FC = 256
NC = F // FC
RS = 32
NLAST = 3
BDEL = 2
LAG_A, LAG_C, LAG_D = 2, 7, 2
O_BX, O_DY, O_AL, O_SP = 0, 196, 392, 588
DQ = D // 4
DD = D // 2
BF = jnp.bfloat16
F32 = jnp.float32
U32 = jnp.uint32
LN_EPS = 1e-5
DEN_EPS = 1e-6
GELU_C0 = 0.7978845608028654
GELU_C1 = 0.044715


def _nn(a, b):
    return lax.dot_general(a, b, (((1,), (0,)), ((), ())), preferred_element_type=F32)


def _nt(a, b):
    return lax.dot_general(a, b, (((1,), (1,)), ((), ())), preferred_element_type=F32)


def _iota(shape, dim):
    return lax.broadcasted_iota(jnp.int32, shape, dim)


def _div28(r):
    return (r * 9363) >> 18


def _fold(x, op):
    f = {jnp.max: jnp.maximum, jnp.min: jnp.minimum, jnp.sum: jnp.add}[op]
    r = op(x, axis=0)
    r = f(r, pltpu.roll(r, 4, 0))
    return f(r, pltpu.roll(r, 2, 0))


def _softmax_pm(p):
    n = p.shape[-1]
    p3 = p.reshape(7, 8, n)
    mx = _fold(p3, jnp.max)
    mn = _fold(p3, jnp.min)
    ep = jnp.exp(p3 - mx[None])
    em = jnp.exp(mn[None] - p3)
    rp = 1.0 / _fold(ep, jnp.sum)
    rm = 1.0 / _fold(em, jnp.sum)
    return ep, em, rp, rm


A_T = [{(0, 0): 1, (1, 1): 1}, {(0, 1): 1, (1, 1): 1}, {(0, 0): 1}, {(1, 1): 1}, {(0, 0): 1, (1, 0): 1},
       {(0, 1): 1, (0, 0): -1}, {(1, 0): 1, (1, 1): -1}]
B_T = [{(0, 0): 1, (1, 1): 1}, {(0, 0): 1}, {(0, 1): 1, (1, 1): -1}, {(1, 0): 1, (0, 0): -1}, {(1, 1): 1},
       {(0, 0): 1, (0, 1): 1}, {(1, 0): 1, (1, 1): 1}]
C_T = [{(0, 0): 1, (1, 1): 1}, {(1, 0): 1, (1, 1): -1}, {(0, 1): 1, (1, 1): 1}, {(0, 0): 1, (1, 0): 1},
       {(0, 1): 1, (0, 0): -1}, {(1, 1): 1}, {(0, 0): 1}]


def _acc(terms):
    terms = sorted(terms, key=lambda p: -p[0])
    z = terms[0][1] if terms[0][0] > 0 else -terms[0][1]
    for sg, v in terms[1:]:
        z = z + v if sg > 0 else z - v
    return z


def _lin(tab, r, get):
    return _acc([(sg, get(i, j)) for (i, j), sg in tab[r].items()])


def _lin2(tab, r1, r2, get):
    terms = [(s1 * s2, get(2 * i1 + i2, 2 * j1 + j2))
             for (i1, j1), s1 in tab[r1].items() for (i2, j2), s2 in tab[r2].items()]
    if len(terms) < 4:
        return _acc(terms)
    return _acc([(1, _acc([terms[0], terms[3]])), terms[1], terms[2]])


def _comb(tab, i, j, get):
    return _acc([(tab[r][(i, j)], get(r)) for r in range(7) if (i, j) in tab[r]])


def _swap64(a, b):
    a = pltpu.bitcast(a, jnp.uint32)
    b = pltpu.bitcast(b, jnp.uint32)
    lo = _iota(a.shape, 1) < 64
    p = jnp.where(lo, a, pltpu.roll(b, 64, 1))
    q = jnp.where(lo, pltpu.roll(a, 64, 1), b)
    return pltpu.bitcast(p, BF), pltpu.bitcast(q, BF)


def _a_list(w):
    w11, w12, w21, w22 = w[:DD, :128], w[:DD, 128:], w[DD:, :128], w[DD:, 128:]
    f = lambda z: z.astype(F32)
    return [(f(w11) + f(w22)).astype(BF), (f(w12) + f(w22)).astype(BF), w11, w22,
            (f(w11) + f(w21)).astype(BF), (f(w12) - f(w11)).astype(BF), (f(w21) - f(w22)).astype(BF)]


def _q_combine(q):
    top = jnp.concatenate([q[0] + q[2] + q[4] - q[5], q[1] + q[5]], axis=1)
    bot = jnp.concatenate([q[4] + q[6], q[0] + q[1] + q[3] - q[6]], axis=1)
    return jnp.concatenate([top, bot], axis=0)


def _kt_rows(w):
    w1, w2 = w[:, :128], w[:, 128:]
    dz = (w1[256:384].astype(F32) - w2[256:384].astype(F32))
    a = jnp.concatenate([w1[:256], dz[64:].astype(BF), w1[384:]], axis=0)
    b = jnp.concatenate([w2[:256], (-dz[:64]).astype(BF), w2[384:]], axis=0)
    y = jnp.concatenate([w1[256:320], w2[320:384]], axis=0)
    return a.T, b.T, y.T


def _kt_form(w1, w2):
    dz = w1[:, 256:384] - w2[:, 256:384]
    y = jnp.concatenate([w1[:, 256:320], w2[:, 320:384]], axis=1)
    a = jnp.concatenate([dz[:, 64:], w1[:, 384:]], axis=1)
    b = jnp.concatenate([-dz[:, :64], w2[:, 384:]], axis=1)
    return y, a, b


def _kt(m01, y, a, b, x):
    m = y.shape[0]
    yy = _nn(y, x[256:384])
    a2 = _nn(a, x[320:])
    b2 = _nn(b, jnp.concatenate([x[256:320], x[384:]], axis=0))
    mm = _nn(m01, x[:256])
    return (yy + a2) + mm[:m], (yy + b2) + mm[m:]


def _feat(col):
    p = (col >= PR).astype(jnp.int32)
    rem = col - p * PR
    return rem >> 1, 2 * p + (rem & 1)


def _words(ref, idx):
    if len(idx) == len(ref.shape) and idx[-2].start is not None:
        idx = idx[:-2] + (slice(idx[-2].start // 2, idx[-2].stop // 2), idx[-1])
    return ref.bitcast(U32), idx


def _ld(ref, *idx):
    view, idx = _words(ref, idx)
    return pltpu.bitcast(view[idx], BF)


def _st(ref, val, *idx):
    if val.dtype == F32:
        ref[idx] = val.astype(BF)
    else:
        view, idx = _words(ref, idx)
        view[idx] = pltpu.bitcast(val, U32)
    return val


def _gate(ref, idx, val):
    w = min(val.shape[1], ref.shape[-1])
    if ref.dtype == BF:
        ref.bitcast(U32)[idx + (slice(0, 8), slice(0, w))] = pltpu.bitcast(val[:8, :w], U32)
    else:
        ref[idx + (slice(0, 8), slice(0, w))] = val[:8, :w]


def _bits(c, fn):
    return (sum(int(fn(r)) << r for r in range(7)) >> c) & 1


def _kernel(xT_h, wqkv_h, wphi_h, wo_h, wg_h, wu_h, wdT_h, dyT_h,
            out_h, dx_h, dwqkv_h, dwphi_h, dwo_h, dwg_h, dwu_h, dwdT_h,
            xT, dyT, wqkv, wphi, wo, w3,
            xnT, xnf, rstd, dyp, doT, phik, vaug,
            wT, w2, k3, lw, wf, bd, bdT,
            kv, kvb, kvT, zb, dkv, dkvb, dkvT, gb,
            ops, cs, bdy, pout, pdx, hr0, hr1, gur, dxs,
            out_o, dx_o, dwqkv_o, dwphi_o, dwo_o, dwgu_o, dwd_o,
            s_x, s_dy, s_w, s_f, so_out, so_dx, so_w, so_g, so_u, so_d):
    cp = pltpu.make_async_copy
    al_ = slice(None)
    q_ = slice(0, DQ)

    def tok(t):
        return pl.ds(pl.multiple_of(t * T, T), T)

    def fch(c):
        return pl.ds(pl.multiple_of(c * FC, FC), FC)

    def cx(t):
        return cp(xT_h.at[:, tok(t)], xT.at[t], s_x.at[t])

    def cdy(t):
        return cp(dyT_h.at[:, tok(t)], dyT.at[t], s_dy.at[t])

    def cf(c, i):
        return cp((wg_h, wu_h, wdT_h)[i].at[:, fch(c)], w3.at[3 * c + i], s_f.at[3 * c + i])

    c_wo = cp(wo_h, wo, s_w.at[0])
    c_wphi = cp(wphi_h, wphi, s_w.at[1])
    c_wqkv = cp(wqkv_h, wqkv, s_w.at[2])

    def o_out(t):
        return cp(out_o.at[t, pl.ds(0, D), :], out_h.at[:, tok(t)], so_out.at[t])

    def o_dx(t):
        return cp(dx_o.at[t, pl.ds(0, D), :], dx_h.at[:, tok(t)], so_dx.at[t])

    def o_g(c):
        return cp(dwgu_o.at[c, :, pl.ds(0, FC)], dwg_h.at[:, fch(c)], so_g.at[c])

    def o_u(c):
        return cp(dwgu_o.at[c, :, pl.ds(FC, FC)], dwu_h.at[:, fch(c)], so_u.at[c])

    def o_d(c):
        return cp(dwd_o.at[c], dwdT_h.at[:, fch(c)], so_d.at[c])

    def o_wo(k):
        return cp(dwo_o.at[k, pl.ds(0, DD), :], dwo_h.at[pl.ds(k * DD, DD), :], so_w.at[2 + k])

    o_wqkv = cp(dwqkv_o.at[0, pl.ds(0, D), :], dwqkv_h, so_w.at[0])
    o_wphi = cp(dwphi_o, dwphi_h, so_w.at[1])

    first = [c_wphi, c_wo, cdy(0), cdy(1), cdy(2), c_wqkv, cdy(3), cx(0), cx(1), cf(0, 0), cx(2), cf(0, 1),
             cx(3), cf(0, 2)]

    def issue(i, carry):
        for k, d in enumerate(first):
            pl.when(i == k)(d.start)
        return carry

    lax.fori_loop(0, len(first), issue, 0)

    lanes = [slice(j * 128, (j + 1) * 128) for j in range(4)]
    rows = lambda i, n: slice(i * n, (i + 1) * n)

    def proj(n, x):
        m01 = jnp.concatenate([_ld(w2, n, 0), _ld(w2, n, 1)], axis=1)
        return _kt(m01, *[_ld(k3, 3 * n + i) for i in range(3)], x)

    def proj_half(n, k, x, yy):
        if k == 0:
            yy = _nn(_ld(k3, 3 * n), x[256:384])
        xa = x[320:] if k == 0 else jnp.concatenate([x[256:320], x[384:]], axis=0)
        m01 = jnp.concatenate([_ld(w2, n, e, rows(k, GR), al_) for e in range(2)], axis=1)
        return yy, (yy + _nn(_ld(k3, 3 * n + 1 + k), xa)) + _nn(m01, x[:256])

    def proj_form(n, w1, w2_):
        for e in range(2):
            _st(w2, jnp.concatenate([w1[:, lanes[e]], w2_[:, lanes[e]]], axis=0), n, e)
        for i, z in enumerate(_kt_form(w1, w2_)):
            _st(k3, z, 3 * n + i)

    def do_tile(t, z):
        z8 = jnp.zeros((8, 128), F32)
        tl = t + z

        def dy_sum(i, m, h):
            get = lambda a, b: _ld(dyp, 4 * tl + 2 * b + m, rows(2 * a + h, DQ), al_).astype(F32)
            _st(bdy, _lin(B_T, (0, 2, 3, 5, 6)[i], get), t, i, m, rows(h, DQ), al_)

        todo = [(i, m, h) for m in range(2) for i in range(5) for h in range(2)]
        dys = [_st(dyp, dyT[t, :, lanes[j]], 4 * t + j) for j in range(4)]
        for n in range(8):
            r = proj(6 + n % 2, dys[n // 2])
            for q in range(4):
                _st(doT, jnp.concatenate([r[q // 2][rows(q % 2, PR)], z8], axis=0), t, n // 2, 4 * (n % 2) + q)
                if n < 5:
                    _gate(dyp, (4 * NT + z,), r[q // 2][rows(q % 2, PR)])
                    dy_sum(*todo.pop(0))
            if n == 0:
                w_back(t, wo[pl.ds(pl.multiple_of(t * GR, 16), GR), :])
            if n == 5:
                _gate(k3, (24 + z,), wf[tl, 0:8, :])

    def b_prep(get, base, r1, t, e):
        lv = {(i, j): _lin(B_T, r1, lambda i1, j1: get(2 * j1 + j, rows(7 * (2 * i1 + i) + e, 16)))
              for i in range(2) for j in range(2)}
        for r2 in range(7):
            _st(ops, _lin(B_T, r2, lambda i, j: lv[i, j]), base + 4 * (7 * r1 + r2) + t, rows(e, 16), al_)

    def w_back(n, w):
        wf[n] = jnp.concatenate([w, jnp.zeros((16, D), w.dtype)], axis=0).T.astype(F32)

    def layer_norm(src, t, j):
        ld = lambda rs: xT[src, rs, lanes[j]].astype(F32)
        mu = jnp.sum(ld(al_), axis=0, keepdims=True) * (1.0 / D)
        yield
        xc = ld(al_) - mu
        var = jnp.sum(xc * xc, axis=0, keepdims=True) * (1.0 / D)
        rs = lax.rsqrt(var + LN_EPS)
        rstd[t, :, lanes[j]] = jnp.broadcast_to(rs, (8, 128))
        for q in range(4):
            yield
            xf = (ld(rows(q, DQ)) - mu) * rs
            xnf[4 * t + j, rows(q, DQ)] = xf
            _st(xnT, xf, 4 * t + j, rows(q, DQ), al_)
        yield

    with jax.named_scope("head0"):
        w3[3 * NC] = jnp.zeros((D, FC), BF)
        c_wphi.wait()
        pw = wphi[...].reshape(DH * H, DH)
        e_m = (_iota((DH, GR), 0) == _feat(_iota((DH, GR), 1))[0]).astype(F32).astype(BF)
        q_m = _nn(pw, e_m)
        keep = (_iota((D, GR), 0) & 3) == _feat(_iota((D, GR), 1))[1]
        q_m = jnp.where(keep, q_m, 0.0).astype(BF)
        r_i = _iota((D, D), 0)
        r_h = _div28(r_i)
        perm = (_iota((D, D), 1) == (r_i - r_h * DH) * H + r_h).astype(F32).astype(BF)
        bdf = _nn(perm, q_m)
        for g in range(NG):
            _st(bd, bdf[rows(g, GR)], g)
            _st(bdT, bdf[rows(g, GR)].T, g)
        c_wo.wait()
        for s in range(2):
            w = wo[rows(s, DD), :].astype(F32)
            proj_form(6 + s, w[:GR], w[GR:])

    def head1(t, carry):
        cdy(t).wait()
        do_tile(t, t >> 3)
        return t

    with jax.named_scope("head1"):
        zh = lax.fori_loop(0, NT - 1, head1, 0) >> 3
    with jax.named_scope("head2"):
        c_wqkv.wait()
        for c in range(1, NC):
            for i in range(3):
                cf(c, i).start()
        cdy(3).wait()
        do_tile(NT - 1, zh)
        wT[:3 * D] = wqkv[...].T
        cx(0).wait()
    with jax.named_scope("head3"):
        for g in range(NG):
            pk = _nn(_ld(bdT, g), wT[rows(NG + g, GR), :])
            vf = wT[rows(2 * NG + g, GR), :].astype(F32)
            w1 = jnp.concatenate([pk[:PR], vf[:PR]], axis=0)
            w2_ = jnp.concatenate([pk[PR:], vf[PR:]], axis=0)
            proj_form(g, w1, w2_)
            wT[rows(4 * NG + g, GR), :] = pk.astype(BF)
        for j in range(4):
            list(layer_norm(0, 0, j))
        pqs = [_nn(_ld(bdT, g), wT[rows(g, GR), :]) for g in range(NG)]
        for s in range(2):
            proj_form(4 + s, pqs[2 * s], pqs[2 * s + 1])
        for g in range(NG):
            if g < 2:
                w_back(NG + g, pqs[g].astype(BF))
            else:
                wT[rows(3 * NG + g, GR), :] = pqs[g].astype(BF)

    def prep_l(src, i):
        a, b, y = _kt_rows(w3[src])
        blks = [a[:, lanes[e]] for e in range(3)] + [b[:, lanes[e]] for e in range(3)] + [y]
        for e, z in enumerate(blks):
            _st(lw, z, 7 * i + e)

    def phase_a(t, carry):
        @pl.when(t < NT - 1)
        def _():
            cx(t + 1).wait()

        @pl.when(t > 0)
        def _():
            cp(wg_h.at[:, fch(0)], w3.at[t - 1], s_f.at[t - 1]).wait()

        ones = jnp.ones((8, 128), F32)
        z = t >> 3
        tn = jnp.minimum(t + 1, NT - 1)
        todo = [(r1, e) for r1 in range(7) for e in range(7)]
        yy, hist = None, []
        for n in range(32):
            j, p = divmod(n, NP)
            yy, r = proj_half(p // 2, p % 2, _ld(xnT, 4 * t + j), yy)
            ep, em, rp, rm = _softmax_pm(r[:PR])
            _st(phik, jnp.concatenate([(ep * rp[None]).reshape(PR, 128), (em * rm[None]).reshape(PR, 128)], axis=0), t, j, p)
            _st(vaug, jnp.concatenate([r[PR:], ones], axis=0), t, j, p)
            if n == 6:
                prep_l(jnp.where(t == 0, 3 * NC, t - 1), jnp.maximum(t - 1, 0))
            if n == 20:
                _gate(k3, (24 + z,), pltpu.bitcast(lw.bitcast(U32)[z, 0:8, :], F32))
            hist.append([r[rows(k, 8)] for k in (7, 10, 13)])
            old = hist[max(n - LAG_A, 0)]
            if p == 0:
                ln = layer_norm(tn, t + 1, j)
            if p in (0, 2, 4, 5, 6, 7):
                _gate(xT, (NT + z,), old[0])
                next(ln)
            for k in range(2 if p < 4 or n == 31 else 1):
                if todo:
                    _gate(xnf, (4 * NT + 4 + z,), old[1 + k])
                    r1, e = todo.pop(0)
                    b_prep(lambda j, rs: xnf[4 * t + j, rs], O_BX, r1, t, e)
        assert not todo
        for p in range(NP):
            cat = lambda ref: jnp.concatenate([_ld(ref, t, j, p) for j in range(4)], axis=1)
            kv[p] = jnp.where(t > 0, kv[p], 0.0) + _nt(cat(vaug), cat(phik))
        return carry

    with jax.named_scope("phaseA"):
        lax.fori_loop(0, NT, phase_a, 0)

    row = _iota((64, GR), 0)
    col_j = _iota((64, GR), 1) & 1
    same_head = (row < PR) & ((row >= DH).astype(jnp.int32) == col_j)

    with jax.named_scope("midA"):
        for c in range(1, NC):
            for i in range(3):
                cf(c, i).wait()

    def ffn(c, carry):
        def act(g, u, dh):
            g2 = g * g
            th = jnp.tanh(g * (GELU_C0 + (GELU_C0 * GELU_C1) * g2))
            hp = 0.5 * th + 0.5
            ge = g * hp
            dge = hp + (g * (1.0 - th * th)) * (0.5 * GELU_C0 + (1.5 * GELU_C0 * GELU_C1) * g2)
            return ge * u, (dh * u) * dge, dh * ge

        def kt(ws, i, x):
            cat = lambda e: jnp.concatenate([_ld(lw, 7 * w + e, rows(i, RS), al_) for w in ws], axis=0)
            m01 = jnp.concatenate([jnp.concatenate([cat(e), cat(3 + e)], axis=0) for e in range(2)], axis=1)
            return _kt(m01, cat(6), cat(2), cat(5), x)

        def s1(t, n, i):
            dhs = kt([2], i, _ld(dyp, 4 * t + n))
            ugs = kt([1, 0], i, _ld(xnT, 4 * t + n))
            for k in range(2):
                h, dg, du = act(ugs[k][RS:], ugs[k][:RS], dhs[k])
                j = 4 * t + n + (c >> 3)
                (hr0 if t < 2 else hr1)[j - 8 * (t // 2), k * 128 + i * RS:k * 128 + (i + 1) * RS] = h
                q, o = divmod(k * 128 + i * RS, 64)
                gur[j, q, o:o + RS] = dg
                gur[j, q, 64 + o:64 + o + RS] = du

        key = lambda r, e: list(A_T[r])[e if len(A_T[r]) > 1 else 0]
        two = lambda r, sg: len(A_T[r]) > 1 and A_T[r][key(r, 1)] == sg

        def a_group(k):
            n = 4 * c + k
            m = (n * 37) >> 8
            r1 = n - 7 * m
            ik = [[_bits(r1, lambda r: key(r, e)[x]) for x in range(2)] for e in range(2)]
            return n, m, ik, (_bits(r1, lambda r: two(r, 1)) - _bits(r1, lambda r: two(r, -1))).astype(F32)

        groups = [a_group(k) for k in range(4)]

        def a_prep(k, e):
            n, m, ik, sg1 = groups[k]
            blk = lambda u, i, k: wf[NG * m + 2 * ik[u][1] + k, pl.ds(pl.multiple_of((2 * ik[u][0] + i) * DQ + 16 * e, 8), 16), :]
            lv = {(i, k): blk(0, i, k) + sg1 * blk(1, i, k) for i in range(2) for k in range(2)}
            for r2 in range(7):
                _st(ops, _lin(A_T, r2, lambda i, k: lv[i, k]), O_AL + 7 * n + r2, rows(e, 16), al_)

        def w_next(k):
            n = jnp.minimum(2 * c + 2 + k, 3 * NG - 1)
            u = n >> 2
            w_back(NG + n, wT[pl.ds(pl.multiple_of((3 - u + 3 * (u >> 1)) * D + (n & 3) * GR, 16), GR), :])

        def dy_prep(r1, t):
            get = lambda i, j: pltpu.bitcast(dyp.bitcast(U32)[4 * t + j, pl.ds(pl.multiple_of(8 * (7 * i + c), 8), 8), :], BF).astype(F32)
            lv = {(i, j): _lin(B_T, r1, lambda i1, j1: get(2 * i1 + i, 2 * j1 + j)) for i in range(2) for j in range(2)}
            for r2 in range(7):
                ops[O_DY + 4 * (7 * r1 + r2) + t + (c >> 3), pl.ds(pl.multiple_of(16 * c, 16), 16), :] = (
                    _lin(B_T, r2, lambda i, j: lv[i, j]).astype(BF))

        dys = [(r1, t) for r1 in range(7) for t in range(NT)]
        for t in range(NT):
            for n in range(4):
                for i in range(128 // RS):
                    s1(t, n, i)
        cn = jnp.minimum(c + 1, NC - 1)
        for i in range(3):
            prep_l(3 * cn + i, i)
        for p in (c, c + 1):
            a = kv[p]
            am = jnp.where(same_head, a, 0.0)
            _st(kvT, am, p)
            _st(kvb, am.T, p)
            zb[p] = jnp.broadcast_to(a.T[:, PR:PR + 1], (GR, 128))

        wq = _swap64(w3[3 * c, :, :128], w3[3 * c + 1, :, :128]) + _swap64(w3[3 * c, :, 128:], w3[3 * c + 1, :, 128:])
        wq = [w.astype(F32) for w in wq]
        ad = _a_list(w3[3 * c + 2])

        def hsum(t, r):
            ref = hr0 if t == 0 else hr1
            return jnp.concatenate([_lin(C_T, r, lambda k, j: ref[4 * e + 2 * j + m, k * 128:(k + 1) * 128])
                                    for e in range(2) for m in range(2)], axis=1).astype(BF)

        def hp(t, r, h):
            po = _nn(ad[r], h)
            pout[7 * t + r] = jnp.where(c > 0, pout[7 * t + r], 0.0) + po[:, :TS]
            pout[7 * t + 7 + r] = jnp.where(c > 0, pout[7 * t + 7 + r], 0.0) + po[:, TS:]

        def b_get(t, r):
            if r in (1, 4):
                return [_ld(dyp, 4 * t + 2 * (r // 4) + m, rows(r // 4, DD), al_) for m in range(2)]
            return [_ld(bdy, t, {0: 0, 2: 1, 3: 2, 5: 3, 6: 4}[r], m) for m in range(2)]

        def hq(t, r, h):
            return _nt(jnp.concatenate(b_get(t, r) + b_get(t + 1, r), axis=1), h)

        qd0 = []
        for r in range(7):
            h = hsum(0, r)
            hp(0, r, h)
            qd0.append(hq(0, r, h))
        q1, qd, hs = [], [], []
        for r1 in range(7):
            q2 = []
            for r2 in range(7):
                r = 7 * r1 + r2
                a = _lin2(A_T, r1, r2, lambda i, k: wq[k][rows(i, DQ)]).astype(BF)
                cc = jnp.concatenate([_lin2(C_T, r1, r2, lambda k, j: gur[4 * t + j, k]) for t in range(NT)], axis=1).astype(BF)
                px = _nn(a, cc)
                for t in range(NT):
                    pdx[49 * t + r] = jnp.where(c > 0, pdx[49 * t + r], 0.0) + px[:, lanes[t]]
                q2.append(_nt(jnp.concatenate([_ld(ops, O_BX + 4 * r + t, q_, al_) for t in range(NT)], axis=1), cc))
                if 7 <= r < 35:
                    a_prep(*divmod(r - 7, 7))
                if r in (35, 38):
                    w_next((r - 35) // 3)
                if r in (41, 44):
                    _gate(ops, (O_SP + (c >> 3),), wf[c >> 3, 0:8, :])
                if r >= 21:
                    dy_prep(*dys.pop(0))
            q1.append({(i, k): _comb(A_T, i, k, lambda r: q2[r]) for i in range(2) for k in range(2)})
            h = hsum(2, r1)
            qd.append(qd0[r1] + hq(2, r1, h))
            if r1 < 7 - NLAST:
                hp(2, r1, h)
            else:
                hs.append((r1, h))
        for k1 in range(2):
            cols = [jnp.concatenate([_comb(A_T, i1, k1, lambda r: q1[r][(i2, k2)])
                                     for i1 in range(2) for i2 in range(2)], axis=0).astype(BF) for k2 in range(2)]
            g_, u_ = _swap64(*cols)
            dwgu_o[c, :, k1 * 128:(k1 + 1) * 128] = g_
            dwgu_o[c, :, FC + k1 * 128:FC + (k1 + 1) * 128] = u_
        dwd_o[c] = _q_combine(qd).astype(BF)
        for r1, h in hs:
            hp(2, r1, h)
        o_g(c).start()
        o_u(c).start()
        o_d(c).start()
        return carry

    with jax.named_scope("ffn"):
        lax.fori_loop(0, NC, ffn, 0)

    def phase_b(t, carry):
        def stage1(s, j, k, yy):
            yy, pq = proj_half(4 + s, k, _ld(xnT, 4 * t + j), yy)
            return yy, [pq[:PR], pq[PR:]]

        def stage2(p, j, pq, dd):
            ep, em, rp, rm = _softmax_pm(pq)
            zp = zb[p, :PR, :].reshape(7, 8, 128)
            zm = zb[p, PR:, :].reshape(7, 8, 128)
            denp = _fold(ep * zp, jnp.sum) * rp
            denm = _fold(em * zm, jnp.sum) * rm
            den = denp + denm + DEN_EPS
            rden = 1.0 / den
            php = ep * (rp * rden)[None]
            phm = em * (rm * rden)[None]
            ph = jnp.concatenate([php.reshape(PR, 128), phm.reshape(PR, 128)], axis=0).astype(BF)
            dp_ = dd[:PR].reshape(7, 8, 128)
            dm_ = dd[PR:].reshape(7, 8, 128)
            ap = _fold(php * dp_, jnp.sum)
            am = _fold(phm * dm_, jnp.sum)
            cc = ap + am
            tp = den * ap - cc * denp
            tm = den * am - cc * denm
            dpq = php * (dp_ - cc[None] * zp - tp[None]) - phm * (dm_ - cc[None] * zm - tm[None])
            xnf[4 * t + j, rows(p, PR)] = dpq.reshape(PR, 128)
            last = jnp.concatenate([_ld(doT, t, j, p, slice(48, 64), al_).astype(F32)[:8], -cc], axis=0).astype(BF)
            return ph, last

        def stage3(p, j, ph, last):
            da = jnp.concatenate([_ld(doT, t, j, p, slice(0, 48), al_), last], axis=0)
            gur[4 * t + j, p // 2, rows(p % 2, PR)] = _nn(_ld(kvT, p), ph)[:PR]
            prev = jnp.where(t > 0, dkv[p], 0.0) if j == 0 else dkv[p]
            dkv[p] = prev + _nt(da, ph)

        items = [(s, j) for j in range(4) for s in range(2)]
        pairs = [(4 * s + q, j) for s, j in items for q in range(4)]
        yy, pqs = stage1(*items[0], 0, None)
        dd = {0: _nn(_ld(kvb, 0), _ld(doT, t, 0, 0))}
        pend = []
        for n, (p, j) in enumerate(pairs):
            i = n // 2 + 1
            if i < 2 * len(items) and n % 2 == 0:
                yy, new = stage1(*items[i // 2], i % 2, yy)
                pqs += new
            if n + 1 < len(pairs):
                dd[n + 1] = _nn(_ld(kvb, pairs[n + 1][0]), _ld(doT, t, pairs[n + 1][1], pairs[n + 1][0]))
            if len(pend) >= BDEL:
                stage3(*pend.pop(0))
            pend.append((p, j) + stage2(p, j, pqs[n], dd[n]))
        for a in pend:
            stage3(*a)
        return carry

    with jax.named_scope("phaseB"):
        lax.fori_loop(0, NT, phase_b, 0)

    with jax.named_scope("midB"):
        keep_dkv = same_head | (row == col_j + PR)
        for p in range(NP):
            a = jnp.where(keep_dkv, dkv[p], 0.0)
            _st(dkvT, a, p)
            _st(dkvb, a.T, p)

    def phase_c(t, carry):
        z = t >> 3
        tl = jnp.minimum(t, NT - 1)

        def strip(g, j):
            for k in range(2):
                p = 2 * g + k
                ph = _ld(phik, t, j, p)
                dphi = _nn(_ld(dkvb, p), _ld(vaug, t, j, p))
                hr0[2 * j + g // 2 + z, pl.ds(g % 2 * 128 + k * PR, PR)] = _nn(_ld(dkvT, p), ph)[:PR]
                phf = ph.astype(F32)
                php = phf[:PR].reshape(7, 8, 128)
                phm = phf[PR:].reshape(7, 8, 128)
                wp = php * dphi[:PR].reshape(7, 8, 128)
                wm = phm * dphi[PR:].reshape(7, 8, 128)
                tp = _fold(wp, jnp.sum)
                tm = _fold(wm, jnp.sum)
                dpk = (wp - wm) - (php * tp[None] - phm * tm[None])
                hr1[2 * j + g // 2 + z, pl.ds(g % 2 * 128 + k * PR, PR)] = dpk.reshape(PR, 128)

        sub = lambda o, e: slice(o + 16 * e, o + 16 * e + 16)
        gets = [lambda k, j, e: gur[4 * t + j, k, sub(0, e)], lambda k, j, e: xnf[4 * t + j, sub(k * GR, e)],
                lambda k, j, e: hr0[2 * j + k // 2, sub(k % 2 * 128, e)], lambda k, j, e: hr1[2 * j + k // 2, sub(k % 2 * 128, e)]]
        seq = [(0, r) for r in range(49)] + [(m, r) for r in range(49) for m in range(1, 4)]
        todo = [(g, j) for g in range(NG) for j in range(4)]

        def c_prep(m, r1, e):
            lv = {(k, j): _lin(C_T, r1, lambda k1, j1: gets[m](2 * k1 + k, 2 * j1 + j, e)) for k in range(2) for j in range(2)}
            for r2 in range(7):
                _st(cs, _lin(C_T, r2, lambda k, j: lv[k, j]), 196 * m + 4 * (7 * r1 + r2) + tl, rows(e, 16), al_)

        after = {n: [] for n in range(-1, len(seq))}
        for r1 in range(7):
            for e in range(7):
                after[max(7 * r1 - 7 + e, -1)].append((0, r1, e))
                for m in range(1, 4):
                    after[28 + 21 * r1 + 7 * (m - 1) + e].append((m, r1, e))
        strip(*todo.pop(0))
        for a in after[-1]:
            c_prep(*a)
        po, px, hist = [], [], []
        spare = [(gur, (4 * NT + z, 0)), (xnf, (4 * NT + 4 + z,)), (hr0, (2 * NT + z,)), (hr1, (2 * NT + z,))]
        for n, (m, r) in enumerate(seq):
            if n % 2 == 1 and todo:
                strip(*todo.pop(0))
            res = _nn(_ld(ops, O_AL + 49 * m + r, q_, q_), _ld(cs, 196 * m + 4 * r + t))
            hist.append(res[:8])
            for a in after[n]:
                if a[0] > 0:
                    _gate(*spare[a[0]], hist[n - LAG_C])
                c_prep(*a)
            po.append(res)
            if m == 0 and r % 7 == 6:
                for i in range(2):
                    for j in range(2):
                        pout[7 * t + r // 7, rows(i, DQ), lanes[j]] += _comb(B_T, i, j, lambda e: po[e])
                po = []
            if m == 3:
                px.append((pdx[49 * t + r] + po[0]) + (po[1] + po[2]))
                po = []
                if r % 7 == 6:
                    for i in range(2):
                        for j in range(2):
                            pdx[49 * t + 7 * (r // 7) + 2 * i + j] = _comb(B_T, i, j, lambda e: px[e])
                    px = []
        return carry

    with jax.named_scope("phaseC"):
        lax.fori_loop(0, NT, phase_c, 0)

    def launch(dma, ref, n, z):
        dma.start()
        view, o = ref.bitcast(U32), ref.shape[1] // 2 - 8
        view[n + z, o:o + 8, 0:128] = jnp.zeros((8, 128), U32)
        return lambda: _gate(ops, (O_SP + z,), pltpu.bitcast(view[n + jnp.minimum(z, 0), o:o + 8, 0:128], F32))

    def finish(t, z):
        hv = [slice(0, 64), slice(64, DQ)]
        sub = lambda i, h: slice(i * DQ + hv[h].start, i * DQ + hv[h].stop)

        def fence(ref, i, h, j):
            v = ref.bitcast(U32)[t + z, pl.ds(sub(i, h).start // 2, 8), lanes[j]]
            _gate(ops, (O_SP + z,), pltpu.bitcast(v, F32))

        def out_part(i, j, h):
            pc = _comb(B_T, i // 2, j // 2, lambda r: pout[7 * t + r, sub(i % 2, h), lanes[j % 2]])
            out_o[t, sub(i, h), lanes[j]] = (xT[t, sub(i, h), lanes[j]].astype(F32) + pc).astype(BF)
            fence(out_o, i, h, j)
            if (i, j, h) == (3, 3, 1):
                launch(o_out(t), out_o, t, z)()

        ms = {}

        def outer(i, j, h):
            dxn = _comb(B_T, i // 2, j // 2, lambda r: pdx[49 * t + 7 * r + 2 * (i % 2) + j % 2, hv[h]])
            dxs[4 * j + i + z, hv[h]] = dxn
            xn = _ld(xnT, 4 * t + j, sub(i, h), al_).astype(F32)
            red = lambda v: jnp.sum(v.reshape(-1, 8, 128), axis=0)
            s1, s2 = red(dxn), red(dxn * xn)
            ms[j] = (s1, s2) if (i, h) == (0, 0) else (ms[j][0] + s1, ms[j][1] + s2)
            _gate(ops, (O_SP + z,), ms[j][0] + ms[j][1] + dxs[4 * j + i, pl.ds(hv[h].start, 8)])

        def dx_part(i, j, h):
            if (i, h) == (0, 0):
                ms[j] = [jnp.sum(v, axis=0, keepdims=True) * (1.0 / D) for v in ms[j]]
            xn = _ld(xnT, 4 * t + j + z, sub(i, h), al_).astype(F32)
            dx = _ld(dyp, 4 * t + j, sub(i, h), al_).astype(F32) + rstd[t, 0:1, lanes[j]] * (
                dxs[4 * j + i, hv[h]] - ms[j][0] - xn * ms[j][1])
            dx_o[t, sub(i, h), lanes[j]] = dx.astype(BF)
            fence(dx_o, i, h, j)
            if (i, j, h) == (3, 3, 1):
                launch(o_dx(t), dx_o, t, z)()

        part = lambda f, *a: lambda: f(*a)
        blocks = lambda gt, f, j: [(gt, part(f, i, j, h)) for i in range(4) for h in range(2)]
        pieces = []
        for j in range(4):
            pieces += blocks((pdx, (49 * NT + z,)), outer, j) + blocks((pout, (7 * NT + z,)), out_part, j)
            pieces += blocks((dxs, (16 + z,)), dx_part, j)
        return pieces

    def run_piece(pieces, hist, q, z, n_per):
        hist.append(q)
        if len(hist) > LAG_D:
            for k, (gt, fn) in enumerate(pieces[:n_per]):
                o = 8 * (k * 14 // n_per)
                _gate(*gt, hist[-1 - LAG_D][o:o + 8])
                fn()
            del pieces[:n_per]

    def q_level(left, right, r1, after):
        q2 = []
        for r2 in range(7):
            q2.append(_nt(jnp.concatenate([left(7 * r1 + r2, t) for t in range(NT)], axis=1),
                          jnp.concatenate([right(7 * r1 + r2, t) for t in range(NT)], axis=1)))
            after(r2, q2[-1])
        return {(i, k): _comb(A_T, i, k, lambda r: q2[r]) for i in range(2) for k in range(2)}

    order = (0, 5, 6, 2, 4, 1, 3)

    def phase_d(m, carry):
        z = m >> 3
        extra = finish(m, z)
        q1, hist = {}, []

        def g_part(i1, k1, i2, k2):
            _st(gb, _comb(A_T, i1, k1, lambda r: q1[r][(i2, k2)]), m, 2 * k1 + k2, rows(2 * i1 + i2, DQ), al_)
            v = gb.bitcast(U32)[m + z, 2 * k1 + k2, pl.ds((2 * i1 + i2) * DQ // 2, 8), :]
            return lambda: _gate(ops, (O_SP + z,), pltpu.bitcast(v, F32))

        parts = [(i1, k1, i2, k2) for i1, k1 in ((1, 0), (0, 0), (0, 1), (1, 1)) for i2 in range(2) for k2 in range(2)]
        for n, r1 in enumerate(order):
            def after(r2, q):
                run_piece(extra, hist, q, z, 3 if 7 * n + r2 < 6 else 2)
                if 36 <= 7 * n + r2 < 48:
                    g_part(*parts.pop(0))()
            q1[r1] = q_level(lambda r, t: _ld(ops, O_BX + 4 * r + t, q_, al_), lambda r, t: _ld(cs, 196 * (m + 1) + 4 * r + t),
                             r1, after)
        assert not extra
        for a in parts:
            g_part(*a)
        return m

    with jax.named_scope("phaseD"):
        z = lax.fori_loop(0, NT - 1, phase_d, 0) >> 3

    with jax.named_scope("tail"):
        def w_grads():
            cols = [pltpu.bitcast(_nt(_ld(gb, m, g), _ld(bd, g)).astype(BF), U32) for m in (0, 2) for g in range(NG)]
            cols += [gb.bitcast(U32)[1, g] for g in range(NG)]
            w = jnp.concatenate(cols, axis=1)
            dwqkv_o[0, :D] = pltpu.bitcast(w, BF)
            return launch(o_wqkv, dwqkv_o, 0, z)

        def phi_grad():
            db = jnp.concatenate([_nn(wT[rows(g, GR), :], _ld(gb, 0, g)) + _nn(wT[rows(NG + g, GR), :], _ld(gb, 2, g))
                                  for g in range(NG)], axis=0)
            keep2 = (_div28(_iota((D, GR), 0)) & 3) == _feat(_iota((D, GR), 1))[1]
            db = jnp.where(keep2, db, 0.0).astype(BF)
            yield
            e_t = (_feat(_iota((GR, DH), 0))[0] == _iota((GR, DH), 1)).astype(F32).astype(BF)
            db = _nn(db, e_t).astype(BF)
            yield
            r_i = _iota((D, D), 0)
            perm_t = (_iota((D, D), 1) == (r_i & 15) * DH + (r_i >> 4)).astype(F32).astype(BF)
            dwphi_o[...] = _nn(perm_t, db).astype(BF).reshape(DH, H, DH)
            o_wphi.start()
            yield

        def wo_grad(k1):
            blk = lambda i1, i2, k2: pltpu.bitcast(_comb(A_T, i1, k1, lambda r: q1[r][(i2, k2)]).astype(BF), U32)
            w = jnp.concatenate([jnp.concatenate([blk(i1, i2, k2) for i1 in range(2) for i2 in range(2)], axis=1)
                                 for k2 in range(2)], axis=0)
            dwo_o[k1, :DD] = pltpu.bitcast(w, BF)
            return launch(o_wo(k1), dwo_o, k1, z) if k1 == 0 else o_wo(k1).start()

        extra = finish(NT - 1, z)
        late = {}
        q1, hist = {}, []
        late[8] = w_grads()
        phi = phi_grad()
        for n, r1 in enumerate(order):
            def after(r2, q):
                run_piece(extra, hist, q, z, 3)
                if 7 * n + r2 in late:
                    late[7 * n + r2]()
            q1[r1] = q_level(lambda r, t: _ld(cs, 4 * r + t), lambda r, t: _ld(ops, O_DY + 4 * r + t, q_, al_), r1, after)
            if 1 <= n <= 3:
                next(phi)
            if n == 4:
                late[43] = wo_grad(0)
        wo_grad(1)

        for t in range(NT):
            o_out(t).wait()
            o_dx(t).wait()
        for c in range(NC):
            o_g(c).wait()
            o_u(c).wait()
            o_d(c).wait()
        o_wqkv.wait()
        o_wphi.wait()
        o_wo(0).wait()
        o_wo(1).wait()


@jax.jit
def pallas_parallel_sum__linear_kernel_hedgehog__glu_gated_geglu__prompt_kernel(
    A_x: jax.Array,
    A_wqkv: jax.Array,
    A_w_phi: jax.Array,
    A_wo: jax.Array,
    B_x: jax.Array,
    B_w_gate: jax.Array,
    B_w_up: jax.Array,
    B_w_down: jax.Array,
    grad_out: jax.Array,
):
    del B_x
    V = pltpu.VMEM
    P = lambda *s: V(s, BF)
    dma = pltpu.SemaphoreType.DMA
    scratch = [
        P(NT + 1, D, T), P(NT, D, T), P(D, 3 * D), P(DH, H, DH), P(D, D), P(3 * NC + 1, D, FC),
        P(4 * NT + 4, D, 128), V((4 * NT + 5, D, 128), F32), V((NT + 1, 8, T), F32), P(4 * NT + 1, D, 128),
        P(NT, 4, NP, 64, 128), P(NT, 4, NP, GR, 128), P(NT, 4, NP, 64, 128),
        P(5 * D, D), P(8, 2, DD, 128), P(25, DQ, 128), P(21, 128, 128), V((4 * NG, D, 128), F32),
        P(NG, GR, GR), P(NG, GR, GR),
        V((NP, 64, GR), F32), P(NP, GR, 64), P(NP, 64, GR), V((NP, GR, 128), F32),
        V((NP, 64, GR), F32), P(NP, GR, 64), P(NP, 64, GR), P(3, NG, D, GR),
        P(O_SP + 1, 128, 128), P(4 * 196, GR, 128), P(NT, 5, 2, DD, 128), V((NT * 7 + 1, DD, TS), F32), V((NT * 49 + 1, DQ, 128), F32),
        V((2 * NT + 1, FC, 128), F32), V((2 * NT + 1, FC, 128), F32), V((4 * NT + 1, 4, 128, 128), F32),
        V((17, DQ, 128), F32),
        V((NT, D + 16, T), BF), V((NT, D + 16, T), BF), V((1, D + 16, 3 * D), BF), V((DH, H, DH), BF), V((2, DD + 16, D), BF),
        V((NC, D, 2 * FC), BF), V((NC, D, FC), BF),
        dma((NT,)), dma((NT,)), dma((3,)), dma((3 * NC,)),
        dma((NT,)), dma((NT,)), dma((4,)), dma((NC,)), dma((NC,)), dma((NC,)),
    ]
    sds = jax.ShapeDtypeStruct
    out_shape = (
        sds((D, S), BF), sds((D, S), BF), sds((D, 3 * D), BF), sds((DH, H, DH), BF), sds((D, D), BF),
        sds((D, F), BF), sds((D, F), BF), sds((D, F), BF),
    )
    hbm = pl.BlockSpec(memory_space=pl.ANY)
    outT, dxT, dwqkv, dwphi, dwo, dwg, dwu, dwdT = pl.pallas_call(
        _kernel,
        out_shape=out_shape,
        in_specs=[hbm] * 8,
        out_specs=(hbm,) * 8,
        scratch_shapes=scratch,
        compiler_params=pltpu.CompilerParams(vmem_limit_bytes=126 * 2 ** 20),
        name="hedgehog_geglu_fwdbwd",
    )(A_x.reshape(S, D).T, A_wqkv, A_w_phi.transpose(1, 0, 2), A_wo, B_w_gate, B_w_up, B_w_down.T,
      grad_out.reshape(S, D).T)
    return (outT.T.reshape(1, S, D), dxT.T.reshape(1, S, D), dwqkv, dwphi.transpose(1, 0, 2), dwo,
            dwg, dwu, dwdT.T)
```
